```python
import jax
import jax.numpy as jnp

def _softmax(x, axis=-1):
    return jax.nn.softmax(x, axis=axis)
def _gelu(x):
    return jax.nn.gelu(x, approximate=True)
def _silu(x):
    return jax.nn.silu(x)
def _sigmoid(x):
    return jax.nn.sigmoid(x)
def _layernorm(x, axis=-1, eps=1e-5):
    m = jnp.mean(x, axis=axis, keepdims=True)
    v = jnp.var(x, axis=axis, keepdims=True)
    return (x - m) / jnp.sqrt(v + eps)
def _scatter_add(tgt, idx, src, axis=0):
    return tgt.at[idx].add(src)
def _segment_sum(src, seg, n):
    return jax.ops.segment_sum(src, seg, n)
class _Rng:
    def __init__(self, key):
        self._k = key
    def _next(self):
        self._k, sub = jax.random.split(self._k)
        return sub
    def normal(self, shape):
        return jax.random.normal(self._next(), shape, dtype=jnp.bfloat16)
    def randint(self, lo, hi, shape):
        return jax.random.randint(self._next(), shape, lo, hi, dtype=jnp.int32)
    def uniform(self, shape, lo=0.0, hi=1.0):
        return jax.random.uniform(self._next(), shape, jnp.bfloat16, lo, hi)
    def permutation(self, n):
        return jax.random.permutation(self._next(), n)


kernel_name = 'standalone__modern_conv_block_convnext_v2__vision'

def setup_inputs():
    _rng = _Rng(jax.random.key(int.from_bytes(__import__("os").urandom(4), "little")))
    _w = (lambda a: (lambda t: t.astype(jnp.bfloat16) if jnp.issubdtype(t.dtype, jnp.floating) else t)(jnp.asarray(a)))
    H = W = 512
    C = 96
    K = 3
    return {
        "x": _w((lambda *s: _rng.normal(s) * 0.05)(1, H, W, C)),
        "dw": _w((lambda *s: _rng.normal(s) * 0.05)(K, K, C)),
        "w1": _w((lambda *s: _rng.normal(s) * 0.05)(C, 4 * C)),
        "w2": _w((lambda *s: _rng.normal(s) * 0.05)(4 * C, C)),
        "grn_gamma": _w((lambda *s: _rng.normal(s) * 0.05)(4 * C)),
        "grn_beta": _w((lambda *s: _rng.normal(s) * 0.05)(4 * C)),
    }

def reference(x, dw, w1, w2, grn_gamma, grn_beta):
    B, H, W, C = x.shape
    K = dw.shape[0]
    pad = K // 2
    xp = jnp.pad(x, ((0,0),(pad,pad),(pad,pad),(0,0)))
    out = jnp.zeros_like(x)
    for i in range(K):
        for j in range(K):
            out = out + xp[:, i:i+H, j:j+W, :] * dw[i, j][None, None, None, :]
    h = _layernorm(out, axis=-1)
    h = jnp.einsum('bhwc,ce->bhwe', h, w1)
    h = _gelu(h)
    gx = jnp.sqrt((h * h).sum(axis=(1, 2), keepdims=True) + 1e-6)
    nx = gx / (gx.mean(axis=-1, keepdims=True) + 1e-6)
    h = grn_gamma * (h * nx) + grn_beta + h
    h = jnp.einsum('bhwe,ec->bhwc', h, w2)
    return x + h
```

```python
import functools
import math
import jax
import jax.numpy as jnp
from jax import lax
import jax.experimental.pallas as pl
import jax.experimental.pallas.tpu as pltpu

C0 = math.sqrt(2.0 / math.pi)
C1 = 0.044715
ALPHA = (C0 * C1) ** (1.0 / 3.0)
K0 = C0 / ALPHA
F32 = jnp.float32
BF16 = jnp.bfloat16

NS = 320
BS = 8
BR = 4
U1 = 1
U2 = 1


def _kernel(x_hbm, dw_ref, w1_ref, w2t_ref, gam_ref, bet_ref, o_hbm,
            h_ref, xin_ref, xr_ref, os_ref, or_ref, s0_ref, s1_ref, a_ref,
            dwb_ref, w1t_ref, w2s_ref, bias_ref, acc_ref,
            sem_in, sem_r, sem_os, sem_or, sem_p, *, H, W, C, E):
    NR = H - NS
    NT = W // 128
    ZROW = 2 * BS

    def in_copy(row0, slot, n=BS):
        return pltpu.make_async_copy(x_hbm.at[pl.ds(row0, n)], xin_ref.at[pl.ds(slot * BS, n)], sem_in.at[slot])

    def r_copy(row0, slot):
        return pltpu.make_async_copy(x_hbm.at[pl.ds(row0, BR)], xr_ref.at[pl.ds(slot * BR, BR)], sem_r.at[slot])

    def os_copy(row0, slot):
        return pltpu.make_async_copy(os_ref.at[pl.ds(slot * BS, BS)], o_hbm.at[pl.ds(row0, BS)], sem_os.at[slot])

    def or_copy(row0, slot):
        return pltpu.make_async_copy(or_ref.at[pl.ds(slot * BR, BR)], o_hbm.at[pl.ds(row0, BR)], sem_or.at[slot])

    P0 = 3 * BR - 2
    pro = pltpu.make_async_copy(x_hbm.at[pl.ds(0, 2)], xr_ref.at[pl.ds(P0, 2)], sem_p.at[0])
    pro.start()
    in_copy(2, 0).start()

    acc_ref[...] = jnp.zeros_like(acc_ref)
    xin_ref[ZROW] = jnp.zeros((C, W), BF16)
    w1t_ref[...] = w1_ref[...].astype(F32).T.astype(BF16)
    for i in range(3):
        dwi = dw_ref[i].astype(F32)
        for j in range(3):
            dwb_ref[i * 3 + j] = jnp.broadcast_to(dwi[j:j + 1, :], (128, C)).T

    def stage_a(xrow):
        lane = lax.broadcasted_iota(jnp.int32, (C, W), 1)
        n = xrow.astype(F32)
        sh = [jnp.where(lane == 0, 0.0, pltpu.roll(n, 1, 1)), n,
              jnp.where(lane == W - 1, 0.0, pltpu.roll(n, W - 1, 1))]

        def cv(i):
            r = None
            for j in range(3):
                t = sh[j] * jnp.tile(dwb_ref[i * 3 + j], (1, NT))
                r = t if r is None else r + t
            return r
        out = s1_ref[...] + cv(2)
        s1_ref[...] = s0_ref[...] + cv(1)
        s0_ref[...] = cv(0)
        m = jnp.sum(out, axis=0, keepdims=True) * (1.0 / C)
        d = out - m
        v = jnp.sum(d * d, axis=0, keepdims=True) * (1.0 / C)
        a_ref[...] = (d * (lax.rsqrt(v + 1e-5) * ALPHA)).astype(BF16)

    def stage_b():
        y = jnp.dot(w1t_ref[...], a_ref[...], preferred_element_type=F32)
        u = (y * y + K0) * y
        return (jnp.tanh(u) + 1.0) * y

    def prologue():
        s0_ref[...] = jnp.zeros_like(s0_ref)
        s1_ref[...] = jnp.zeros_like(s1_ref)

        def body(t, _):
            stage_a(xr_ref[P0 + t])
            return 0
        lax.fori_loop(0, 2, body, 0)

    pro.wait()
    prologue()
    nblk = H // BS

    def p1(i, _):
        h0 = i * U1
        blk = h0 // BS
        slot = blk % 2

        @pl.when(h0 % BS == 0)
        def _():
            @pl.when(blk < nblk - 1)
            def _():
                in_copy(2 + blk * BS, slot).wait()

            @pl.when(blk == nblk - 1)
            def _():
                in_copy(H - BS + 2, (nblk - 1) % 2, BS - 2).wait()

            @pl.when(blk < nblk - 2)
            def _():
                in_copy(2 + (blk + 1) * BS, 1 - slot).start()

            @pl.when(blk == nblk - 2)
            def _():
                in_copy(H - BS + 2, (nblk - 1) % 2, BS - 2).start()

        for u in range(U1):
            h = h0 + u
            g = stage_b()
            g2 = g * g
            s = g2[:, 0:128]
            for t in range(1, NT):
                s = s + g2[:, t * 128:(t + 1) * 128]
            acc_ref[...] += s
            h_ref[jnp.maximum(h - NR, 0)] = g.astype(BF16)
            stage_a(xin_ref[jnp.where(h + 2 < H, slot * BS + h % BS, ZROW)])
        return 0
    lax.fori_loop(0, H // U1, p1, 0)

    in_copy(NR, 0).start()
    r_copy(2, 0).start()
    s = jnp.sum(acc_ref[...].T, axis=0, keepdims=True) * (1.0 / (4.0 * ALPHA * ALPHA))
    gx = jnp.sqrt(s + 1e-6)
    nx = gx / (jnp.sum(gx, axis=1, keepdims=True) * (1.0 / E) + 1e-6)
    gam = gam_ref[...].astype(F32).reshape(1, E)
    bet = bet_ref[...].astype(F32).reshape(1, E)
    w2t = w2t_ref[...].astype(F32)
    w2s_ref[...] = (w2t * ((gam * nx + 1.0) * (1.0 / (2.0 * ALPHA)))).astype(BF16)
    bias_ref[...] = jnp.broadcast_to(jnp.sum(w2t * bet, axis=1, keepdims=True), bias_ref.shape)

    prologue()

    def proj(g, xrow):
        o = jnp.dot(w2s_ref[...], g, preferred_element_type=F32)
        return (o + (jnp.tile(bias_ref[...], (1, NT)) + xrow.astype(F32))).astype(BF16)

    nrb = NR // BR
    nsb = NS // BS

    def p2(with_s, i, _):
        k0 = i * U2
        rb = k0 // BR
        par = rb % 2

        @pl.when(k0 % BR == 0)
        def _():
            r_copy(2 + rb * BR, rb % 3).wait()

            @pl.when(rb < nrb - 1)
            def _():
                r_copy(2 + (rb + 1) * BR, (rb + 1) % 3).start()

            @pl.when(rb >= 2)
            def _():
                or_copy((rb - 2) * BR, par).wait()
            if with_s:
                in_copy(NR + rb * BS, par).wait()

                @pl.when(rb < nsb - 1)
                def _():
                    in_copy(NR + (rb + 1) * BS, 1 - par).start()

                @pl.when(rb >= 2)
                def _():
                    os_copy(NR + (rb - 2) * BS, par).wait()

        for u in range(U2):
            k = k0 + u
            g = stage_b().astype(BF16)
            if with_s:
                for q in range(2):
                    r = par * BS + (k % BR) * 2 + q
                    os_ref[r] = proj(h_ref[2 * k + q], xin_ref[r])
            or_ref[par * BR + k % BR] = proj(g, xr_ref[(k + 3 * BR - 2) % (3 * BR)])
            stage_a(xr_ref[k % (3 * BR)])

        @pl.when((k0 + U2) % BR == 0)
        def _():
            or_copy(rb * BR, par).start()
            if with_s:
                os_copy(NR + rb * BS, par).start()
        return 0
    lax.fori_loop(0, NS // 2 // U2, functools.partial(p2, True), 0)
    lax.fori_loop(NS // 2 // U2, NR // U2, functools.partial(p2, False), 0)
    for b in (nsb - 2, nsb - 1):
        os_copy(NR + b * BS, b % 2).wait()
    for b in (nrb - 2, nrb - 1):
        or_copy(b * BR, b % 2).wait()


@jax.jit
def pallas_standalone__modern_conv_block_convnext_v2__vision_kernel(x, dw, w1, w2, grn_gamma, grn_beta):
    B, H, W, C = x.shape
    E = w1.shape[1]
    xt = jnp.transpose(x, (0, 1, 3, 2)).reshape(H, C, W)
    vm = pl.BlockSpec(memory_space=pltpu.VMEM)
    out = pl.pallas_call(
        functools.partial(_kernel, H=H, W=W, C=C, E=E),
        in_specs=[pl.BlockSpec(memory_space=pl.ANY), vm, vm, vm, vm, vm],
        out_specs=pl.BlockSpec(memory_space=pl.ANY),
        out_shape=jax.ShapeDtypeStruct((H, C, W), x.dtype),
        scratch_shapes=[
            pltpu.VMEM((NS, E, W), BF16),
            pltpu.VMEM((2 * BS + 1, C, W), BF16),
            pltpu.VMEM((3 * BR, C, W), BF16),
            pltpu.VMEM((2 * BS, C, W), BF16),
            pltpu.VMEM((2 * BR, C, W), BF16),
            pltpu.VMEM((C, W), F32),
            pltpu.VMEM((C, W), F32),
            pltpu.VMEM((C, W), BF16),
            pltpu.VMEM((9, C, 128), F32),
            pltpu.VMEM((E, C), BF16),
            pltpu.VMEM((C, E), BF16),
            pltpu.VMEM((C, 128), F32),
            pltpu.VMEM((E, 128), F32),
            pltpu.SemaphoreType.DMA((2,)),
            pltpu.SemaphoreType.DMA((3,)),
            pltpu.SemaphoreType.DMA((2,)),
            pltpu.SemaphoreType.DMA((2,)),
            pltpu.SemaphoreType.DMA((1,)),
        ],
        compiler_params=pltpu.CompilerParams(
            vmem_limit_bytes=128 * 1024 * 1024,
        ),
        name="convnext",
    )(xt, dw, w1, w2.T, grn_gamma, grn_beta)
    return jnp.transpose(out.reshape(B, H, C, W), (0, 1, 3, 2))
```

```python
import functools
import math
import jax
import jax.numpy as jnp
from jax import lax
import jax.experimental.pallas as pl
import jax.experimental.pallas.tpu as pltpu

C0 = math.sqrt(2.0 / math.pi)
C1 = 0.044715
ALPHA = (C0 * C1) ** (1.0 / 3.0)
K0 = C0 / ALPHA
F32 = jnp.float32
BF16 = jnp.bfloat16
U32 = jnp.uint32

BS = 8
REC = (1, 2, 3)
KEEP = (0, 4, 5, 6, 7)
NI = 4
NO = 2
FOLD = 1
SD = 2
CD = 0
CNT = '011212121100-011212121100-012222000'
N0 = 3
PT = 1
TK = 1
ORD = 'M45R-M67R-M0R'


def _kernel(x_hbm, dw_ref, w1_ref, w2t_ref, gam_ref, bet_ref, o_hbm,
            h_ref, xi_ref, xo_ref, dwb_ref, w1t_ref, cv_ref, bias_ref, z_ref,
            sem_i, sem_o, *, H, W, C, E):
    NT = W // 128
    G = C // 8
    NE = E // 128
    NB = H // BS

    def shift(v, right, zero):
        lane = lax.broadcasted_iota(jnp.int32, (v.shape[0], 128), 1)
        rl = [pltpu.roll(v[:, t * 128:(t + 1) * 128], 1 if right else 127, 1) for t in range(NT)]
        edge, step = (0, 1) if right else (127, -1)
        return jnp.concatenate(
            [jnp.where(lane == edge, rl[t - step] if 0 <= t - step < NT else zero, rl[t]) for t in range(NT)], axis=1)

    def mlp_in(a, lo, hi):
        a = jnp.concatenate([a, jnp.zeros((128 - C, W), BF16)], axis=0)
        y = jnp.dot(pltpu.bitcast(w1t_ref[lo // 2:hi // 2], BF16), a, preferred_element_type=F32)
        u = (y * y + K0) * y
        return (jnp.tanh(u) + 1.0) * y

    ST = 2 * NT * C
    W2 = ST + 2 * 64

    def put_cv(ho, lo, v):
        for t in range(NT):
            r = (ho * NT + t) * C + lo
            cv_ref[r:r + v.shape[0]] = v[:, 128 * t:128 * t + 128]

    def get_cv(ho, lo, n):
        return jnp.concatenate([cv_ref[(ho * NT + t) * C + lo:(ho * NT + t) * C + lo + n] for t in range(NT)], axis=1)

    def add_stats(ho, vs, first):
        for k, v in enumerate(vs):
            for t in range(NT):
                r = ST + 64 * k + 8 * (ho * NT + t)
                p = v[:, 128 * t:128 * t + 128]
                cv_ref[r:r + 8] = p if first else cv_ref[r:r + 8] + p

    def ln_stats(mr_ref, n):
        tot = []
        for k in range(2):
            v = [cv_ref[pl.ds(ST + 64 * k + j, n, stride=8)] for j in range(8)]
            tot.append((((v[0] + v[1]) + (v[2] + v[3])) + ((v[4] + v[5]) + (v[6] + v[7]))) * (1.0 / C))
        var = jnp.maximum(tot[1] - tot[0] * tot[0], 0.0)
        if not FOLD:
            mr_ref[0:n] = tot[0]
        mr_ref[8:8 + n] = lax.rsqrt(var + 1e-5) * ALPHA

    def ln_apply(v, mr_ref, q):
        def bc(k):
            return jnp.concatenate([jnp.broadcast_to(mr_ref[k + q + t:k + q + t + 1], (v.shape[0], 128))
                                    for t in range(NT)], axis=1)
        if not FOLD:
            v = v - bc(0)
        return (v * bc(8)).astype(BF16)

    def in2(b):
        return pltpu.make_async_copy(x_hbm.at[pl.ds(b * BS, BS)], xi_ref.at[b % NI], sem_i.at[b % NI])

    def out2(b):
        return pltpu.make_async_copy(xo_ref.at[pl.ds((b % NO) * BS, BS)], o_hbm.at[pl.ds(b * BS, BS)], sem_o.at[b % NO])

    def in1(b):
        row = jnp.minimum(BS - 1 + b * BS, H - BS)
        return pltpu.make_async_copy(x_hbm.at[pl.ds(row, BS)], xo_ref.at[pl.ds((b % 2) * BS, BS)], sem_o.at[b % 2])

    def pass1(sh_ref, mr_ref, ab_ref, au_ref, dwm_ref, acc_ref):
        pro = pltpu.make_async_copy(x_hbm.at[pl.ds(0, BS - 1)], xo_ref.at[pl.ds(BS + 1, BS - 1)], sem_o.at[1])
        pro.start()
        in1(0).start()
        for b in range(NI - 1):
            in2(b).start()

        z_ref[0] = 0
        acc_ref[...] = jnp.zeros_like(acc_ref)
        xo_ref[BS] = jnp.zeros((G, 8, W), BF16)
        xo_ref[2 * BS] = jnp.zeros((G, 8, W), BF16)
        w1f = w1_ref[...].astype(F32)
        if FOLD:
            w1f = w1f - jnp.sum(w1f, axis=0, keepdims=True) * (1.0 / C)
        w1p = jnp.concatenate([w1f, jnp.zeros((128 - C, E), F32)], axis=0)
        w1t_ref[...] = pltpu.bitcast(w1p.T.astype(BF16), U32)
        for i in range(3):
            dwi = dw_ref[i].astype(F32)
            for j in range(3):
                dwb_ref[i * 3 + j] = jnp.broadcast_to(dwi[j:j + 1, :], (128, C)).T
        col = lax.broadcasted_iota(jnp.int32, (8, 128), 1) - lax.broadcasted_iota(jnp.int32, (8, 128), 0)
        for g in range(G):
            halves = []
            for ho in range(2):
                m = jnp.zeros((8, 128), F32)
                for i in range(3):
                    for j in range(3):
                        r = ho + i
                        m = jnp.where(col == (r // 2) * 48 + j * 16 + (r % 2) * 8,
                                      dwb_ref[i * 3 + j, 8 * g:8 * g + 8], m)
                halves.append(m)
            dwm_ref[g] = pltpu.bitcast(jnp.concatenate(halves, axis=0).astype(BF16), U32)

        def shift_stage(slot, row, par, g):
            xc = pltpu.bitcast(xo_ref[pl.ds(slot * BS + row, 2), g].reshape(16, W), U32)
            sh_ref[par, g, 0] = shift(xc, True, jnp.uint32(0))
            sh_ref[par, g, 1] = xc
            sh_ref[par, g, 2] = shift(xc, False, jnp.uint32(0))

        def conv_stage(par, c):
            o = []
            for g in (2 * c, 2 * c + 1):
                rhs = jnp.concatenate([sh_ref[p, g, j] for p in (par, 1 - par) for j in range(3)]
                                      + [jnp.zeros((16, W), U32)], axis=0)
                og = jnp.dot(pltpu.bitcast(dwm_ref[g], BF16), pltpu.bitcast(rhs, BF16), preferred_element_type=F32)
                put_cv(0, 8 * g, og[0:8])
                put_cv(1, 8 * g, og[8:16])
                o.append(og)
            vs = (o[0] + o[1], o[0] * o[0] + o[1] * o[1])
            for ho in range(2):
                add_stats(ho, [v[8 * ho:8 * ho + 8] for v in vs], c == 0)

        def scale_stage(par, c):
            for ho in range(2):
                ab_ref[ho, 16 * c:16 * c + 16] = ln_apply(get_cv(ho, 16 * c, 16), mr_ref, ho * NT)
                au_ref[par, ho, 8 * c:8 * c + 8] = pltpu.bitcast(ab_ref[ho, 16 * c:16 * c + 16], U32)

        pro.wait()
        for i in range(4):
            if i == 3:
                ln_stats(mr_ref, 2 * NT)
            for c in range(G // 2):
                if i == 3:
                    scale_stage(0, c)
                if i == 2 or (i == 3 and c < G // 2 - CD):
                    conv_stage(i % 2, c)
                if i < 3 or c < G // 2 - CD:
                    for g in (2 * c, 2 * c + 1):
                        shift_stage(1, 2 * i, i % 2, g)
        keep_ref = xo_ref

        def body(b, _):
            in1(b).wait()
            pend = []
            for s in range(BS // 2):
                for c in range(2 * NE):
                    ho, e = divmod(c, NE)
                    gl = mlp_in(pltpu.bitcast(au_ref[s % 2, ho], BF16), 128 * e, 128 * e + 128)
                    g2 = gl * gl
                    sq = g2[:, 0:128]
                    for t in range(1, NT):
                        sq = sq + g2[:, t * 128:(t + 1) * 128]
                    acc_ref[128 * e:128 * e + 128] += sq
                    if 2 * s + ho in KEEP:
                        h_ref[b, KEEP.index(2 * s + ho), 128 * e:128 * e + 128] = gl.astype(BF16)
                    ss, cc = divmod(s * 2 * NE + c - CD, 2 * NE)
                    if cc == 0:
                        ln_stats(mr_ref, 2 * NT)
                    scale_stage(1 - ss % 2, cc)
                    conv_stage(ss % 2, cc)
                    for g in (2 * cc, 2 * cc + 1):
                        if ss < 0:
                            pend.append(((b + 1) % 2, BS - 2, 1, g))
                        else:
                            pend.append((b % 2, jnp.where(b == NB - 1, BS - 1, 2 * ss), ss % 2, g))
                    while len(pend) > 2 * (SD - 1):
                        shift_stage(*pend.pop(0))
                if s == 0:
                    @pl.when(b < NB - 1)
                    def _():
                        in1(b + 1).start()
            for p in pend:
                shift_stage(*p)
            return 0
        lax.fori_loop(0, NB, body, 0)

        s = jnp.sum(acc_ref[...].T, axis=0, keepdims=True) * (1.0 / (4.0 * ALPHA * ALPHA))
        gx = jnp.sqrt(s + 1e-6)
        nx = gx / (jnp.sum(gx, axis=1, keepdims=True) * (1.0 / E) + 1e-6)
        gam = gam_ref[...].astype(F32).reshape(1, E)
        bet = bet_ref[...].astype(F32).reshape(1, E)
        w2t = w2t_ref[...].astype(F32)
        w2s = pltpu.bitcast((w2t * ((gam * nx + 1.0) * (1.0 / (2.0 * ALPHA)))).astype(BF16), F32)
        for k in range(NE):
            cv_ref[W2 + k * (C // 2):W2 + (k + 1) * (C // 2)] = w2s[:, 128 * k:128 * k + 128]
        bias_ref[...] = jnp.broadcast_to(jnp.sum(w2t * bet, axis=1, keepdims=True), bias_ref.shape)

    pl.run_scoped(pass1, pltpu.VMEM((2, G, 3, 8, W), U32), pltpu.VMEM((16, 128), F32),
                  pltpu.VMEM((2, C, W), BF16), pltpu.VMEM((2, 2, C // 2, W), U32), pltpu.VMEM((G, 8, 128), U32),
                  pltpu.VMEM((E, 128), F32))

    def pass2(ps_ref, xf_ref, mr_ref, a_ref, g_ref):
        def conv_piece(slot, r, g):
            c = slice(8 * g, 8 * g + 8)
            rows = []
            for i in range(r - 1, r + 2):
                if r == REC[0] or i == r + 1:
                    n = xi_ref[slot, i, g].astype(F32)
                    if REC[0] <= i <= REC[-1]:
                        xf_ref[i - REC[0], c] = n
                else:
                    n = xf_ref[i - REC[0], c]
                rows.append(n)
            T = []
            for j in range(3):
                t = None
                for i in range(3):
                    p = rows[i] * jnp.tile(dwb_ref[i * 3 + j, c], (1, NT))
                    t = p if t is None else t + p
                T.append(t)
            o = shift(T[0], True, 0.0) + T[1] + shift(T[2], False, 0.0)
            put_cv(0, 8 * g, o)
            add_stats(0, (o, o * o), g == 0)

            if g == G - 1:
                ln_stats(mr_ref, NT)
                a_ref[r - REC[0]] = ln_apply(get_cv(0, 0, C), mr_ref, 0)

        in2(0).wait()
        for r in REC:
            for g in range(G):
                conv_piece(0, r, g)

        def body(b, _):
            @pl.when(b + NI - 1 < NB)
            def _():
                in2(b + NI - 1).start()

            @pl.when(b + 1 < NB)
            def _():
                in2(b + 1).wait()

            @pl.when(b >= NO)
            def _():
                out2(b - NO).wait()
            nxt = jnp.minimum(b + 1, NB - 1) % NI
            z = z_ref[0]
            done = [0]

            def release(v, n):
                if n:
                    if v is not None:
                        dwb_ref[9, pl.ds(pl.multiple_of(8 * z, 8), 8)] = v[-8:, -128:]
                    for _ in range(n):
                        conv_piece(nxt, REC[done[0] // G], done[0] % G)
                        done[0] += 1

            release(None, N0)
            for r, ops, cnt in zip(REC, ORD.split('-'), CNT.split('-')):
                cnt = [int(c) for c in cnt]
                for op in ops:
                    if op == 'M':
                        gl = mlp_in(a_ref[r - REC[0]], 0, E)
                        g_ref[...] = gl.astype(BF16)
                        for k in range(NE):
                            release(gl[128 * k:128 * k + 128], cnt.pop(0))
                        continue
                    row = r if op == 'R' else int(op)
                    if PT == 1:
                        for t2 in range(NT // 2):
                            res = xi_ref[b % NI, row, :, :, 256 * t2:256 * t2 + 256].astype(F32).reshape(C, 256)
                            os_ = []
                            for t in (2 * t2, 2 * t2 + 1):
                                ts = slice(128 * t, 128 * t + 128)
                                g = g_ref[:, ts] if op == 'R' else h_ref[b, KEEP.index(row), :, ts]
                                w = jnp.concatenate([cv_ref[W2 + k * (C // 2):W2 + (k + 1) * (C // 2)]
                                                     for k in range(NE)], axis=1)
                                os_.append(jnp.dot(pltpu.bitcast(w, BF16), g, preferred_element_type=F32) + bias_ref[...])
                                if t != 2:
                                    release(os_[-1][:8 * TK], cnt.pop(0))
                            o = jnp.concatenate(os_, axis=1) + res
                            xo_ref[(b % NO) * BS + row, :, :, 256 * t2:256 * t2 + 256] = o.reshape(G, 8, 256).astype(BF16)
                        continue
                    for k in range(NE):
                        ks = slice(128 * k, 128 * k + 128)
                        g = g_ref[ks] if op == 'R' else h_ref[b, KEEP.index(row), ks]
                        w = cv_ref[W2 + k * (C // 2):W2 + (k + 1) * (C // 2)]
                        d = jnp.dot(pltpu.bitcast(w, BF16), g, preferred_element_type=F32)
                        if k == 0:
                            o = (d + jnp.tile(bias_ref[...], (1, NT))) + xi_ref[b % NI, row].astype(F32).reshape(C, W)
                        else:
                            o = (ps_ref[...] if PT == 2 else o) + d
                        if PT == 2 and k < NE - 1:
                            ps_ref[...] = o
                        release(o[:8 * TK], cnt.pop(0))
                    xo_ref[(b % NO) * BS + row] = o.reshape(G, 8, W).astype(BF16)
                assert not cnt and done[0] < (r - REC[0] + 2) * G
            assert done[0] == len(REC) * G, done
            out2(b).start()
            return 0
        lax.fori_loop(0, NB, body, 0)
        for b in range(NB - NO, NB):
            out2(b).wait()

    pl.run_scoped(pass2, pltpu.VMEM((C, W), F32), pltpu.VMEM((len(REC), C, W), F32), pltpu.VMEM((16, 128), F32),
                  pltpu.VMEM((len(REC), C, W), BF16), pltpu.VMEM((E, W), BF16))


@jax.jit
def pallas_standalone__modern_conv_block_convnext_v2__vision_kernel(x, dw, w1, w2, grn_gamma, grn_beta):
    B, H, W, C = x.shape
    E = w1.shape[1]
    G = C // 8
    xt = jnp.transpose(x, (0, 1, 3, 2)).reshape(H, G, 8, W)
    vm = pl.BlockSpec(memory_space=pltpu.VMEM)
    out = pl.pallas_call(
        functools.partial(_kernel, H=H, W=W, C=C, E=E),
        in_specs=[pl.BlockSpec(memory_space=pl.ANY), vm, vm, vm, vm, vm],
        out_specs=pl.BlockSpec(memory_space=pl.ANY),
        out_shape=jax.ShapeDtypeStruct((H, G, 8, W), x.dtype),
        scratch_shapes=[
            pltpu.VMEM((H // BS, len(KEEP), E, W), BF16),
            pltpu.VMEM((NI, BS, G, 8, W), BF16),
            pltpu.VMEM((NO * BS + 1, G, 8, W), BF16),
            pltpu.VMEM((10, C, 128), F32),
            pltpu.VMEM((E // 2, 128), U32),
            pltpu.VMEM((2 * (W // 128) * C + 128 + (E // 128) * C // 2, 128), F32),
            pltpu.VMEM((C, 128), F32),
            pltpu.SMEM((1,), jnp.int32),
            pltpu.SemaphoreType.DMA((NI,)),
            pltpu.SemaphoreType.DMA((NO,)),
        ],
        compiler_params=pltpu.CompilerParams(
            vmem_limit_bytes=128 * 1024 * 1024,
            disable_bounds_checks=True,
        ),
        name="convnext",
    )(xt, dw, w1, w2.T, grn_gamma, grn_beta)
    return jnp.transpose(out.reshape(B, H, C, W), (0, 1, 3, 2))
```

```python
import functools
import math
import jax
import jax.numpy as jnp
from jax import lax
import jax.experimental.pallas as pl
import jax.experimental.pallas.tpu as pltpu

C0 = math.sqrt(2.0 / math.pi)
C1 = 0.044715
ALPHA = (C0 * C1) ** (1.0 / 3.0)
K0 = C0 / ALPHA
F32 = jnp.float32
BF16 = jnp.bfloat16
U32 = jnp.uint32

BS = 8
REC = (1, 2, 3)
KEEP = (0, 4, 5, 6, 7)
NI = 4
NO = 2
SD = 2
N0 = 3
TK = 1
PT = 1
ORD = 'M45R-M67R-M0R'
CNT = '011212121100-011212121100-012222000'


def _kernel(x_hbm, dw_ref, w1_ref, w2t_ref, gam_ref, bet_ref, o_hbm,
            h_ref, xi_ref, xo_ref, dwb_ref, w1t_ref, w2s_ref, bias_ref, z_ref,
            sem_i, sem_o, *, H, W, C, E):
    NT = W // 128
    G = C // 8
    NE = E // 128
    NB = H // BS
    B1 = 2 * BS
    N1 = H // B1

    def shift(v, right, zero):
        lane = lax.broadcasted_iota(jnp.int32, (v.shape[0], 128), 1)
        rl = [pltpu.roll(v[:, t * 128:(t + 1) * 128], 1 if right else 127, 1) for t in range(NT)]
        edge, step = (0, 1) if right else (127, -1)
        return jnp.concatenate(
            [jnp.where(lane == edge, rl[t - step] if 0 <= t - step < NT else zero, rl[t]) for t in range(NT)], axis=1)

    def mlp_in(a, lo, hi):
        a = jnp.concatenate([a, jnp.zeros((128 - C, W), BF16)], axis=0)
        y = jnp.dot(pltpu.bitcast(w1t_ref[lo // 2:hi // 2], BF16), a, preferred_element_type=F32)
        u = (y * y + K0) * y
        return (jnp.tanh(u) + 1.0) * y

    def add_stats(st, q, vs, first):
        for k, v in enumerate(vs):
            for t in range(NT):
                r = 8 * (q + t)
                p = v[:, 128 * t:128 * t + 128]
                st[k, r:r + 8] = p if first else st[k, r:r + 8] + p

    def ln_stats(st, mr_ref, n):
        tot = []
        for k in range(2):
            v = [st[k, pl.ds(j, n, stride=8)] for j in range(8)]
            tot.append((((v[0] + v[1]) + (v[2] + v[3])) + ((v[4] + v[5]) + (v[6] + v[7]))) * (1.0 / C))
        var = jnp.maximum(tot[1] - tot[0] * tot[0], 0.0)
        r = lax.rsqrt(var + 1e-5) * ALPHA
        for q in range(n):
            mr_ref[q] = jnp.broadcast_to(r[q:q + 1], (8, 128))

    def ln_apply(v, mr_ref, q):
        r = jnp.concatenate([mr_ref[q + t] for t in range(NT)], axis=1)
        return (v * jnp.tile(r, (v.shape[0] // 8, 1))).astype(BF16)

    def in1(b):
        row = jnp.minimum(BS - 1 + b * B1, H - B1)
        return pltpu.make_async_copy(x_hbm.at[pl.ds(row, B1)], xi_ref.at[pl.ds((b % 2) * B1, B1)], sem_o.at[b % 2])

    def in2(b):
        return pltpu.make_async_copy(x_hbm.at[pl.ds(b * BS, BS)], xi_ref.at[pl.ds((b % NI) * BS, BS)], sem_i.at[b % NI])

    def out2(b):
        return pltpu.make_async_copy(xo_ref.at[b % NO], o_hbm.at[pl.ds(b * BS, BS)], sem_o.at[b % NO])

    def pass1(sh_ref, cv_ref, st_ref, mr_ref, au_ref, dwm_ref, acc_ref):
        pro = pltpu.make_async_copy(x_hbm.at[pl.ds(0, BS - 1)], xi_ref.at[pl.ds(B1 + 1, BS - 1)], sem_o.at[1])
        pro.start()
        in1(0).start()

        z_ref[0] = 0
        acc_ref[...] = jnp.zeros_like(acc_ref)
        xi_ref[B1] = jnp.zeros((G, 8, W), BF16)
        xi_ref[2 * B1] = jnp.zeros((G, 8, W), BF16)
        w1f = w1_ref[...].astype(F32)
        w1f = w1f - jnp.sum(w1f, axis=0, keepdims=True) * (1.0 / C)
        w1p = jnp.concatenate([w1f, jnp.zeros((128 - C, E), F32)], axis=0)
        w1t_ref[...] = pltpu.bitcast(w1p.T.astype(BF16), U32)
        for i in range(3):
            dwi = dw_ref[i].astype(F32)
            for j in range(3):
                dwb_ref[(i * 3 + j) * C:(i * 3 + j + 1) * C] = jnp.broadcast_to(dwi[j:j + 1, :], (128, C)).T
        col = lax.broadcasted_iota(jnp.int32, (8, 128), 1) - lax.broadcasted_iota(jnp.int32, (8, 128), 0)
        for g in range(G):
            halves = []
            for ho in range(2):
                m = jnp.zeros((8, 128), F32)
                for i in range(3):
                    for j in range(3):
                        r = ho + i
                        m = jnp.where(col == (r // 2) * 48 + j * 16 + (r % 2) * 8,
                                      dwb_ref[pl.ds((i * 3 + j) * C + 8 * g, 8)], m)
                halves.append(m)
            dwm_ref[g] = pltpu.bitcast(jnp.concatenate(halves, axis=0).astype(BF16), U32)

        def shift_stage(row, par, g):
            xc = pltpu.bitcast(xi_ref[pl.ds(row, 2), g].reshape(16, W), U32)
            sh_ref[par, g, 0] = shift(xc, True, jnp.uint32(0))
            sh_ref[par, g, 1] = xc
            sh_ref[par, g, 2] = shift(xc, False, jnp.uint32(0))

        def cv_row(par, g):
            return 8 * g + (C if (g < 2 and par) else 0)

        held = []

        def conv_stage(par, g):
            rhs = jnp.concatenate([sh_ref[p, g, j] for p in (par, 1 - par) for j in range(3)]
                                  + [jnp.zeros((16, W), U32)], axis=0)
            o = jnp.dot(pltpu.bitcast(dwm_ref[g], BF16), pltpu.bitcast(rhs, BF16), preferred_element_type=F32)
            for ho in range(2):
                cv_ref[ho, pl.ds(cv_row(par, g), 8)] = o[8 * ho:8 * ho + 8]
            if g % 2 == 0:
                held.append(o)
                return
            p = held.pop()
            vs = (p + o, p * p + o * o)
            for ho in range(2):
                add_stats(st_ref.at[par], ho * NT, [v[8 * ho:8 * ho + 8] for v in vs], g == 1)

        def scale_stage(par, g):
            for ho in range(2):
                v = ln_apply(cv_ref[ho, pl.ds(cv_row(par, g), 16)], mr_ref, ho * NT)
                au_ref[par, ho, 4 * g:4 * g + 8] = pltpu.bitcast(v, U32)

        pro.wait()
        for i in range(4):
            if i == 3:
                ln_stats(st_ref.at[0], mr_ref, 2 * NT)
            for g in range(G):
                if i == 3 and g % 2 == 0:
                    scale_stage(0, g)
                if i >= 2:
                    conv_stage(i % 2, g)
                shift_stage(B1 + 2 * i, i % 2, g)

        def body(b, _):
            in1(b).wait()

            @pl.when(b < N1 - 1)
            def _():
                in1(b + 1).start()

            @pl.when(b == N1 - 1)
            def _():
                in2(0).start()
                in2(1).start()
            pend = []
            for s in range(B1 // 2):
                par = s % 2
                row = (b % 2) * B1 + jnp.where(b == N1 - 1, min(2 * s + BS - 1, B1 - 1), 2 * s)
                for g in range(G):
                    ho, e = divmod(g, G // 2)
                    lo, hi = e * 2 * E // G, (e + 1) * 2 * E // G
                    gl = mlp_in(pltpu.bitcast(au_ref[par, ho], BF16), lo, hi)
                    g2 = gl * gl
                    sq = g2[:, 0:128]
                    for t in range(1, NT):
                        sq = sq + g2[:, t * 128:(t + 1) * 128]
                    acc_ref[lo:hi] += sq
                    blk, r = divmod(2 * s + ho, BS)
                    if r in KEEP:
                        h_ref[2 * b + blk, KEEP.index(r), lo:hi] = gl.astype(BF16)
                    if g == 0:
                        ln_stats(st_ref.at[1 - par], mr_ref, 2 * NT)
                    if g % 2 == 0:
                        scale_stage(1 - par, g)
                    conv_stage(par, g)
                    pend.append((row, par, g))
                    while len(pend) > SD:
                        shift_stage(*pend.pop(0))
            for p in pend:
                shift_stage(*p)
            return 0
        lax.fori_loop(0, N1, body, 0)
        in2(2).start()

        s = jnp.sum(acc_ref[...].T, axis=0, keepdims=True) * (1.0 / (4.0 * ALPHA * ALPHA))
        gx = jnp.sqrt(s + 1e-6)
        nx = gx / (jnp.sum(gx, axis=1, keepdims=True) * (1.0 / E) + 1e-6)
        gam = gam_ref[...].astype(F32).reshape(1, E)
        bet = bet_ref[...].astype(F32).reshape(1, E)
        w2t = w2t_ref[...].astype(F32)
        w2s_ref[...] = pltpu.bitcast((w2t * ((gam * nx + 1.0) * (1.0 / (2.0 * ALPHA)))).astype(BF16), U32)
        bias_ref[...] = jnp.broadcast_to(jnp.sum(w2t * bet, axis=1, keepdims=True), bias_ref.shape)

    pl.run_scoped(pass1, pltpu.VMEM((2, G, 3, 8, W), U32), pltpu.VMEM((2, C + 16, W), F32),
                  pltpu.VMEM((2, 2, 16 * NT, 128), F32), pltpu.VMEM((2 * NT, 8, 128), F32),
                  pltpu.VMEM((2, 2, C // 2, W), U32), pltpu.VMEM((G, 8, 128), U32),
                  pltpu.VMEM((E, 128), F32))

    def pass2(xf_ref, cv_ref, st_ref, mr_ref, a_ref, g_ref):
        def conv_piece(slot, r, g):
            c = slice(8 * g, 8 * g + 8)
            rows = []
            for i in range(r - 1, r + 2):
                if r == REC[0] or i == r + 1:
                    n = xi_ref[slot * BS + i, g].astype(F32)
                    if REC[0] <= i <= REC[-1]:
                        xf_ref[i - REC[0], c] = n
                else:
                    n = xf_ref[i - REC[0], c]
                rows.append(n)
            T = []
            for j in range(3):
                t = None
                for i in range(3):
                    p = rows[i] * jnp.tile(dwb_ref[pl.ds((i * 3 + j) * C + 8 * g, 8)], (1, NT))
                    t = p if t is None else t + p
                T.append(t)
            o = shift(T[0], True, 0.0) + T[1] + shift(T[2], False, 0.0)
            cv_ref[c] = o
            add_stats(st_ref, 0, (o, o * o), g == 0)
            if g == G - 1:
                ln_stats(st_ref, mr_ref, NT)
                a_ref[r - REC[0]] = ln_apply(cv_ref[...], mr_ref, 0)

        in2(0).wait()
        for r in REC:
            for g in range(G):
                conv_piece(0, r, g)

        def body(b, _):
            @pl.when(b + 1 < NB)
            def _():
                in2(b + 1).wait()

            @pl.when(b >= NO)
            def _():
                out2(b - NO).wait()

            @pl.when(b + NI - 1 < NB)
            def _():
                in2(b + NI - 1).start()
            nxt = jnp.minimum(b + 1, NB - 1) % NI
            z = z_ref[0]
            done = [0]

            def release(v, n):
                n = min(n, len(REC) * G - done[0])
                if n:
                    if v is not None:
                        dwb_ref[pl.ds(pl.multiple_of(9 * C + 8 * z, 8), 8)] = v[-8:, -128:]
                    for _ in range(n):
                        conv_piece(nxt, REC[done[0] // G], done[0] % G)
                        done[0] += 1

            release(None, N0)
            for r, ops, cnt in zip(REC, ORD.split('-'), CNT.split('-')):
                cnt = [int(c) for c in cnt]
                for op in ops:
                    if op == 'M':
                        gl = mlp_in(a_ref[r - REC[0]], 0, E)
                        g_ref[...] = gl.astype(BF16)
                        for k in range(NE):
                            release(gl[128 * k:128 * k + 128], cnt.pop(0))
                        continue
                    row = r if op == 'R' else int(op)
                    for t2 in range(NT // 2):
                        ws = slice(256 * t2, 256 * t2 + 256)
                        res = xi_ref[(b % NI) * BS + row, :, :, ws].astype(F32).reshape(C, 256)
                        os_ = []
                        for t in (2 * t2, 2 * t2 + 1):
                            ts = slice(128 * t, 128 * t + 128)
                            g = g_ref[:, ts] if op == 'R' else h_ref[b, KEEP.index(row), :, ts]
                            os_.append(jnp.dot(pltpu.bitcast(w2s_ref[...], BF16), g, preferred_element_type=F32)
                                       + bias_ref[...])
                            if t != 2:
                                release(os_[-1][:8 * TK], cnt.pop(0))
                        o = jnp.concatenate(os_, axis=1) + res
                        xo_ref[b % NO, row, :, :, ws] = o.reshape(G, 8, 256).astype(BF16)
                assert not cnt and done[0] < (r - REC[0] + 2) * G
            assert done[0] == len(REC) * G, done
            out2(b).start()
            return 0
        lax.fori_loop(0, NB, body, 0)
        for b in range(NB - NO, NB):
            out2(b).wait()

    pl.run_scoped(pass2, pltpu.VMEM((len(REC), C, W), F32), pltpu.VMEM((C, W), F32),
                  pltpu.VMEM((2, 8 * NT, 128), F32), pltpu.VMEM((NT, 8, 128), F32),
                  pltpu.VMEM((len(REC), C, W), BF16), pltpu.VMEM((E, W), BF16))


@jax.jit
def pallas_standalone__modern_conv_block_convnext_v2__vision_kernel(x, dw, w1, w2, grn_gamma, grn_beta):
    B, H, W, C = x.shape
    E = w1.shape[1]
    G = C // 8
    xt = jnp.transpose(x, (0, 1, 3, 2)).reshape(H, G, 8, W)
    vm = pl.BlockSpec(memory_space=pltpu.VMEM)
    out = pl.pallas_call(
        functools.partial(_kernel, H=H, W=W, C=C, E=E),
        in_specs=[pl.BlockSpec(memory_space=pl.ANY), vm, vm, vm, vm, vm],
        out_specs=pl.BlockSpec(memory_space=pl.ANY),
        out_shape=jax.ShapeDtypeStruct((H, G, 8, W), x.dtype),
        scratch_shapes=[
            pltpu.VMEM((H // BS, len(KEEP), E, W), BF16),
            pltpu.VMEM((NI * BS + 1, G, 8, W), BF16),
            pltpu.VMEM((NO, BS, G, 8, W), BF16),
            pltpu.VMEM((9 * C + 8, 128), F32),
            pltpu.VMEM((E // 2, 128), U32),
            pltpu.VMEM((C // 2, E), U32),
            pltpu.VMEM((C, 128), F32),
            pltpu.SMEM((1,), jnp.int32),
            pltpu.SemaphoreType.DMA((NI,)),
            pltpu.SemaphoreType.DMA((NO,)),
        ],
        compiler_params=pltpu.CompilerParams(
            vmem_limit_bytes=128 * 1024 * 1024,
            disable_bounds_checks=True,
        ),
        name="convnext",
    )(xt, dw, w1, w2.T, grn_gamma, grn_beta)
    return jnp.transpose(out.reshape(B, H, C, W), (0, 1, 3, 2))
```

```python
import functools
import math
import jax
import jax.numpy as jnp
from jax import lax
import jax.experimental.pallas as pl
import jax.experimental.pallas.tpu as pltpu

C0 = math.sqrt(2.0 / math.pi)
C1 = 0.044715
ALPHA = (C0 * C1) ** (1.0 / 3.0)
K0 = C0 / ALPHA
F32 = jnp.float32
BF16 = jnp.bfloat16
U32 = jnp.uint32

BS = 8
REC = (1, 2, 3)
KEEP = (0, 4, 5, 6, 7)
NI = 4
NO = 2
SD = 2
N0 = 0
RD = 1
WD = 1
TK = 1
PT = 1
ORD = 'M45R-M67R-M0R'
CNT = '100321120110-100321221211-011220110'


def _kernel(x_hbm, dw_hbm, w1_hbm, w2t_hbm, gam_hbm, bet_hbm, o_hbm,
            h_ref, xi_ref, xo_ref, dwb_ref, w1t_ref, w2s_ref, bias_ref, z_ref,
            sem_i, sem_o, sem_w, *, H, W, C, E):
    NT = W // 128
    G = C // 8
    NE = E // 128
    NB = H // BS
    B1 = 2 * BS
    N1 = H // B1

    def shift(v, right, zero):
        lane = lax.broadcasted_iota(jnp.int32, (v.shape[0], 128), 1)
        rl = [pltpu.roll(v[:, t * 128:(t + 1) * 128], 1 if right else 127, 1) for t in range(NT)]
        edge, step = (0, 1) if right else (127, -1)
        return jnp.concatenate(
            [jnp.where(lane == edge, rl[t - step] if 0 <= t - step < NT else zero, rl[t]) for t in range(NT)], axis=1)

    def mlp_in(a, lo, hi):
        a = jnp.concatenate([a, jnp.zeros((128 - C, W), BF16)], axis=0)
        y = jnp.dot(pltpu.bitcast(w1t_ref[lo // 2:hi // 2], BF16), a, preferred_element_type=F32)
        u = (y * y + K0) * y
        return (jnp.tanh(u) + 1.0) * y

    def add_stats(st, q, vs, first):
        for k, v in enumerate(vs):
            for t in range(NT):
                r = 8 * (q + t)
                p = v[:, 128 * t:128 * t + 128]
                st[k, r:r + 8] = p if first else st[k, r:r + 8] + p

    def ln_stats(st, mr_ref, n):
        tot = []
        for k in range(2):
            v = [st[k, pl.ds(j, n, stride=8)] for j in range(8)]
            tot.append((((v[0] + v[1]) + (v[2] + v[3])) + ((v[4] + v[5]) + (v[6] + v[7]))) * (1.0 / C))
        var = jnp.maximum(tot[1] - tot[0] * tot[0], 0.0)
        r = lax.rsqrt(var + 1e-5) * ALPHA
        for q in range(n):
            mr_ref[q] = jnp.broadcast_to(r[q:q + 1], (8, 128))

    def ln_apply(v, mr_ref, q):
        r = jnp.concatenate([mr_ref[q + t] for t in range(NT)], axis=1)
        return (v * jnp.tile(r, (v.shape[0] // 8, 1))).astype(BF16)

    def in1(b):
        row = jnp.minimum(BS - 1 + b * B1, H - B1)
        return pltpu.make_async_copy(x_hbm.at[pl.ds(row, B1)], xi_ref.at[pl.ds((b % 2) * B1, B1)], sem_o.at[b % 2])

    def in2(b):
        return pltpu.make_async_copy(x_hbm.at[pl.ds(b * BS, BS)], xi_ref.at[pl.ds((b % NI) * BS, BS)], sem_i.at[b % NI])

    def out2(b):
        return pltpu.make_async_copy(xo_ref.at[b % NO], o_hbm.at[pl.ds(b * BS, BS)], sem_o.at[b % NO])

    def pass1(sh_ref, cv_ref, st_ref, mr_ref, au_ref, dwm_ref, acc_ref, w1_ref, w2t_ref, dw_ref, gam_ref, bet_ref):
        pro = pltpu.make_async_copy(x_hbm.at[pl.ds(0, BS - 1)], xi_ref.at[pl.ds(B1 + 1, BS - 1)], sem_o.at[1])
        wts = [pltpu.make_async_copy(src, dst, sem_w.at[k]) for k, (src, dst) in enumerate(
            zip((dw_hbm, w1_hbm, w2t_hbm, gam_hbm, bet_hbm), (dw_ref, w1_ref, w2t_ref, gam_ref, bet_ref)))]
        wts[0].start()
        wts[1].start()
        pro.start()
        in1(0).start()
        for cp in wts[2:]:
            cp.start()

        z_ref[0] = 0
        acc_ref[...] = jnp.zeros_like(acc_ref)
        xi_ref[B1] = jnp.zeros((G, 8, W), BF16)
        xi_ref[2 * B1] = jnp.zeros((G, 8, W), BF16)
        wts[0].wait()
        wts[1].wait()
        w1f = w1_ref[...].astype(F32)
        w1f = w1f - jnp.sum(w1f, axis=0, keepdims=True) * (1.0 / C)
        w1p = jnp.concatenate([w1f, jnp.zeros((128 - C, E), F32)], axis=0)
        w1t_ref[...] = pltpu.bitcast(w1p.T.astype(BF16), U32)
        for i in range(3):
            dwi = dw_ref[i].astype(F32)
            for j in range(3):
                dwb_ref[(i * 3 + j) * C:(i * 3 + j + 1) * C] = jnp.broadcast_to(dwi[j:j + 1, :], (128, C)).T
        col = lax.broadcasted_iota(jnp.int32, (8, 128), 1) - lax.broadcasted_iota(jnp.int32, (8, 128), 0)
        for g in range(G):
            halves = []
            for ho in range(2):
                m = jnp.zeros((8, 128), F32)
                for i in range(3):
                    for j in range(3):
                        r = ho + i
                        m = jnp.where(col == (r // 2) * 48 + j * 16 + (r % 2) * 8,
                                      dwb_ref[pl.ds((i * 3 + j) * C + 8 * g, 8)], m)
                halves.append(m)
            dwm_ref[g] = pltpu.bitcast(jnp.concatenate(halves, axis=0).astype(BF16), U32)

        def shift_stage(row, par, g):
            xc = pltpu.bitcast(xi_ref[pl.ds(row, 2), g].reshape(16, W), U32)
            sh_ref[par, g, 0] = shift(xc, True, jnp.uint32(0))
            sh_ref[par, g, 1] = xc
            sh_ref[par, g, 2] = shift(xc, False, jnp.uint32(0))

        def cv_row(par, g):
            return 8 * g + (C if (g < 2 and par) else 0)

        held = []

        def conv_stage(par, g):
            rhs = jnp.concatenate([sh_ref[p, g, j] for p in (par, 1 - par) for j in range(3)]
                                  + [jnp.zeros((16, W), U32)], axis=0)
            o = jnp.dot(pltpu.bitcast(dwm_ref[g], BF16), pltpu.bitcast(rhs, BF16), preferred_element_type=F32)
            for ho in range(2):
                cv_ref[ho, pl.ds(cv_row(par, g), 8)] = o[8 * ho:8 * ho + 8]
            if g % 2 == 0:
                held.append(o)
                return
            p = held.pop()
            vs = (p + o, p * p + o * o)
            for ho in range(2):
                add_stats(st_ref.at[par], ho * NT, [v[8 * ho:8 * ho + 8] for v in vs], g == 1)

        def scale_stage(par, g):
            for ho in range(2):
                v = ln_apply(cv_ref[ho, pl.ds(cv_row(par, g), 16)], mr_ref, ho * NT)
                au_ref[par, ho, 4 * g:4 * g + 8] = pltpu.bitcast(v, U32)

        pro.wait()
        for i in range(4):
            if i == 3:
                ln_stats(st_ref.at[0], mr_ref, 2 * NT)
            for g in range(G):
                if i == 3 and g % 2 == 0:
                    scale_stage(0, g)
                if i >= 2:
                    conv_stage(i % 2, g)
                shift_stage(B1 + 2 * i, i % 2, g)

        def body(b, _):
            in1(b).wait()

            @pl.when(b < N1 - 1)
            def _():
                in1(b + 1).start()

            @pl.when(b == N1 - 1)
            def _():
                in2(0).start()
                in2(1).start()
            pend = []
            for s in range(B1 // 2):
                par = s % 2
                row = (b % 2) * B1 + jnp.where(b == N1 - 1, min(2 * s + BS - 1, B1 - 1), 2 * s)
                for g in range(G):
                    ho, e = divmod(g, G // 2)
                    lo, hi = e * 2 * E // G, (e + 1) * 2 * E // G
                    gl = mlp_in(pltpu.bitcast(au_ref[par, ho], BF16), lo, hi)
                    g2 = gl * gl
                    sq = g2[:, 0:128]
                    for t in range(1, NT):
                        sq = sq + g2[:, t * 128:(t + 1) * 128]
                    acc_ref[lo:hi] += sq
                    blk, r = divmod(2 * s + ho, BS)
                    if r in KEEP:
                        h_ref[2 * b + blk, KEEP.index(r), lo:hi] = gl.astype(BF16)
                    if g == 0:
                        ln_stats(st_ref.at[1 - par], mr_ref, 2 * NT)
                    if g % 2 == 0:
                        scale_stage(1 - par, g)
                    conv_stage(par, g)
                    pend.append((row, par, g))
                    while len(pend) > SD:
                        shift_stage(*pend.pop(0))
            for p in pend:
                shift_stage(*p)
            return 0
        lax.fori_loop(0, N1, body, 0)
        in2(2).start()
        for cp in wts[2:]:
            cp.wait()

        s = jnp.sum(acc_ref[...].T, axis=0, keepdims=True) * (1.0 / (4.0 * ALPHA * ALPHA))
        gx = jnp.sqrt(s + 1e-6)
        nx = gx / (jnp.sum(gx, axis=1, keepdims=True) * (1.0 / E) + 1e-6)
        gam = gam_ref[...].astype(F32).reshape(1, E)
        bet = bet_ref[...].astype(F32).reshape(1, E)
        w2t = w2t_ref[...].astype(F32)
        w2s_ref[...] = pltpu.bitcast((w2t * ((gam * nx + 1.0) * (1.0 / (2.0 * ALPHA)))).astype(BF16), U32)
        bias_ref[...] = jnp.broadcast_to(jnp.sum(w2t * bet, axis=1, keepdims=True), bias_ref.shape)

    pl.run_scoped(pass1, pltpu.VMEM((2, G, 3, 8, W), U32), pltpu.VMEM((2, C + 16, W), F32),
                  pltpu.VMEM((2, 2, 16 * NT, 128), F32), pltpu.VMEM((2 * NT, 8, 128), F32),
                  pltpu.VMEM((2, 2, C // 2, W), U32), pltpu.VMEM((G, 8, 128), U32),
                  pltpu.VMEM((E, 128), F32),
                  *[pltpu.VMEM(r.shape, r.dtype) for r in (w1_hbm, w2t_hbm, dw_hbm, gam_hbm, bet_hbm)])

    def pass2(xf_ref, cv_ref, st_ref, mr_ref, a_ref, g_ref):
        def conv_piece(slot, r, g):
            c = slice(8 * g, 8 * g + 8)
            rows = []
            for i in range(r - 1, r + 2):
                if r == REC[0] or i == r + 1:
                    n = xi_ref[slot * BS + i, g].astype(F32)
                    if REC[0] <= i <= REC[-1]:
                        xf_ref[i - REC[0], c] = n
                else:
                    n = xf_ref[i - REC[0], c]
                rows.append(n)
            T = []
            for j in range(3):
                t = None
                for i in range(3):
                    p = rows[i] * jnp.tile(dwb_ref[pl.ds((i * 3 + j) * C + 8 * g, 8)], (1, NT))
                    t = p if t is None else t + p
                T.append(t)
            o = shift(T[0], True, 0.0) + T[1] + shift(T[2], False, 0.0)
            cv_ref[c] = o
            add_stats(st_ref, 0, (o, o * o), g == 0)
            if g == G - 1:
                ln_stats(st_ref, mr_ref, NT)
                a_ref[r - REC[0]] = ln_apply(cv_ref[...], mr_ref, 0)

        in2(0).wait()
        for r in REC:
            for g in range(G):
                conv_piece(0, r, g)

        def body(b, _):
            @pl.when(b + 1 < NB)
            def _():
                in2(b + 1).wait()

            @pl.when(b >= NO)
            def _():
                out2(b - NO).wait()

            @pl.when(b + NI - 1 < NB)
            def _():
                in2(b + NI - 1).start()
            nxt = jnp.minimum(b + 1, NB - 1) % NI
            z = z_ref[0]
            done = [0]

            def release(v, n):
                n = min(n, len(REC) * G - done[0])
                if n:
                    if v is not None:
                        dwb_ref[pl.ds(pl.multiple_of(9 * C + 8 * z, 8), 8)] = v[-8:, -128:]
                    for _ in range(n):
                        conv_piece(nxt, REC[done[0] // G], done[0] % G)
                        done[0] += 1

            release(None, N0)
            for r, ops, cnt in zip(REC, ORD.split('-'), CNT.split('-')):
                cnt = [int(c) for c in cnt]
                for op in ops:
                    if op == 'M':
                        gl = mlp_in(a_ref[r - REC[0]], 0, E)
                        g_ref[...] = gl.astype(BF16)
                        for k in range(NE):
                            release(gl[128 * k:128 * k + 128], cnt.pop(0))
                        continue
                    row = r if op == 'R' else int(op)
                    for t2 in range(NT // 2):
                        ws = slice(256 * t2, 256 * t2 + 256)
                        res = xi_ref[(b % NI) * BS + row, :, :, ws].astype(F32).reshape(C, 256)
                        os_ = []
                        for t in (2 * t2, 2 * t2 + 1):
                            ts = slice(128 * t, 128 * t + 128)
                            g = g_ref[:, ts] if op == 'R' else h_ref[b, KEEP.index(row), :, ts]
                            os_.append(jnp.dot(pltpu.bitcast(w2s_ref[...], BF16), g, preferred_element_type=F32)
                                       + bias_ref[...])
                            if t != 2:
                                release(os_[-1][:8 * TK], cnt.pop(0))
                        o = jnp.concatenate(os_, axis=1) + res
                        xo_ref[b % NO, row, :, :, ws] = o.reshape(G, 8, 256).astype(BF16)
                    if RD:
                        pltpu.make_async_copy(xo_ref.at[b % NO, row], o_hbm.at[b * BS + row], sem_o.at[b % NO]).start()
                assert not cnt and done[0] < (r - REC[0] + 2) * G
            assert done[0] == len(REC) * G, done
            if not RD:
                out2(b).start()
            return 0
        lax.fori_loop(0, NB, body, 0)
        for b in range(NB - NO, NB):
            out2(b).wait()

    pl.run_scoped(pass2, pltpu.VMEM((len(REC), C, W), F32), pltpu.VMEM((C, W), F32),
                  pltpu.VMEM((2, 8 * NT, 128), F32), pltpu.VMEM((NT, 8, 128), F32),
                  pltpu.VMEM((len(REC), C, W), BF16), pltpu.VMEM((E, W), BF16))


@jax.jit
def pallas_standalone__modern_conv_block_convnext_v2__vision_kernel(x, dw, w1, w2, grn_gamma, grn_beta):
    B, H, W, C = x.shape
    E = w1.shape[1]
    G = C // 8
    xt = jnp.transpose(x, (0, 1, 3, 2)).reshape(H, G, 8, W)
    out = pl.pallas_call(
        functools.partial(_kernel, H=H, W=W, C=C, E=E),
        in_specs=[pl.BlockSpec(memory_space=pl.ANY)] * 6,
        out_specs=pl.BlockSpec(memory_space=pl.ANY),
        out_shape=jax.ShapeDtypeStruct((H, G, 8, W), x.dtype),
        scratch_shapes=[
            pltpu.VMEM((H // BS, len(KEEP), E, W), BF16),
            pltpu.VMEM((NI * BS + 1, G, 8, W), BF16),
            pltpu.VMEM((NO, BS, G, 8, W), BF16),
            pltpu.VMEM((9 * C + 8, 128), F32),
            pltpu.VMEM((E // 2, 128), U32),
            pltpu.VMEM((C // 2, E), U32),
            pltpu.VMEM((C, 128), F32),
            pltpu.SMEM((1,), jnp.int32),
            pltpu.SemaphoreType.DMA((NI,)),
            pltpu.SemaphoreType.DMA((NO,)),
            pltpu.SemaphoreType.DMA((5,)),
        ],
        compiler_params=pltpu.CompilerParams(
            vmem_limit_bytes=128 * 1024 * 1024,
            disable_bounds_checks=True,
        ),
        name="convnext",
    )(xt, dw, w1, w2.T, grn_gamma, grn_beta)
    return jnp.transpose(out.reshape(B, H, C, W), (0, 1, 3, 2))
```

```python
import functools
import math

import jax
import jax.numpy as jnp
from jax import lax
import jax.experimental.pallas as pl
import jax.experimental.pallas.tpu as pltpu

F32 = jnp.float32
BF16 = jnp.bfloat16
U32 = jnp.uint32

_C0 = math.sqrt(2.0 / math.pi)
_C1 = 0.044715
ALPHA = (_C0 * _C1) ** (1.0 / 3.0)
K0 = _C0 / ALPHA

BS = 8
REC = (1, 2, 3)
KEEP = (0, 4, 5, 6, 7)
NI = 4
NO = 2
UNROLL1 = 4
UNROLL2 = 4
KEPT_WITH = ((4, 5), (6, 7), (0,))
PIECES = '100321120110-100321221211-011220110'.split('-')


def _kernel(x_hbm, dw_hbm, w1_hbm, w2t_hbm, gam_hbm, bet_hbm, o_hbm,
            h_ref, xi_ref, xo_ref, dwb_ref, w1t_ref, w2s_ref, bias_ref, z_ref,
            sem_i, sem_o, sem_w, *, H, W, C, E):
    NT = W // 128
    G = C // 8
    NB = H // BS

    def tile(v, t):
        return v[:, 128 * t:128 * (t + 1)]

    def tap(i, j, g):
        return dwb_ref[pl.ds((i * 3 + j) * C + 8 * g, 8)]

    def shift(v, right, zero):
        lane = lax.broadcasted_iota(jnp.int32, (v.shape[0], 128), 1)
        rl = [pltpu.roll(tile(v, t), 1 if right else 127, 1) for t in range(NT)]
        edge, step = (0, 1) if right else (127, -1)
        return jnp.concatenate(
            [jnp.where(lane == edge, rl[t - step] if 0 <= t - step < NT else zero, rl[t])
             for t in range(NT)], axis=1)

    def add_stats(st, q, vs, first):
        for k, v in enumerate(vs):
            for t in range(NT):
                r = pl.ds(8 * (q + t), 8)
                st[k, r] = tile(v, t) if first else st[k, r] + tile(v, t)

    def ln_stats(st, rs_ref, n):
        mom = []
        for k in range(2):
            v = [st[k, pl.ds(j, n, stride=8)] for j in range(8)]
            mom.append((((v[0] + v[1]) + (v[2] + v[3])) + ((v[4] + v[5]) + (v[6] + v[7]))) * (1.0 / C))
        var = jnp.maximum(mom[1] - mom[0] * mom[0], 0.0)
        r = lax.rsqrt(var + 1e-5) * ALPHA
        for q in range(n):
            rs_ref[q] = jnp.broadcast_to(r[q:q + 1], (8, 128))

    def ln_scale(v, rs_ref, q):
        r = jnp.concatenate([rs_ref[q + t] for t in range(NT)], axis=1)
        return (v * jnp.tile(r, (v.shape[0] // 8, 1))).astype(BF16)

    def mlp_in(a, lo, hi):
        a = jnp.concatenate([a, jnp.zeros((128 - C, W), BF16)], axis=0)
        y = jnp.dot(pltpu.bitcast(w1t_ref[lo // 2:hi // 2], BF16), a, preferred_element_type=F32)
        return (jnp.tanh((y * y + K0) * y) + 1.0) * y

    def load(row, n, slot, off=0):
        return pltpu.make_async_copy(
            x_hbm.at[pl.ds(row, n)], xi_ref.at[pl.ds(slot * BS + off, n)], sem_i.at[slot])

    def in1(b):
        return load(jnp.minimum(b * BS + BS - 1, H - BS), BS, NI - 2 + b % 2)

    def in2(b):
        return load(b * BS, BS, b % NI)

    def out2(b):
        return pltpu.make_async_copy(xo_ref.at[b % NO], o_hbm.at[pl.ds(b * BS, BS)], sem_o.at[b % NO])

    def pass1(sh_ref, cv_ref, st_ref, rs_ref, a_ref, dwm_ref, acc_ref,
              w1_ref, w2t_ref, dw_ref, gam_ref, bet_ref):
        wts = [pltpu.make_async_copy(src, dst, sem_w.at[k]) for k, (src, dst) in enumerate(
            zip((dw_hbm, w1_hbm, w2t_hbm, gam_hbm, bet_hbm), (dw_ref, w1_ref, w2t_ref, gam_ref, bet_ref)))]
        head = load(0, BS - 1, NI - 1, 1)
        wts[0].start()
        wts[1].start()
        head.start()
        in1(0).start()
        for cp in wts[2:]:
            cp.start()
        for b in range(NI - 2):
            in2(b).start()

        z_ref[0] = 0
        acc_ref[...] = jnp.zeros_like(acc_ref)
        xi_ref[(NI - 1) * BS] = jnp.zeros((G, 8, W), BF16)
        xi_ref[NI * BS] = jnp.zeros((G, 8, W), BF16)
        wts[0].wait()
        wts[1].wait()
        w1 = w1_ref[...].astype(F32)
        w1 = w1 - jnp.sum(w1, axis=0, keepdims=True) * (1.0 / C)
        w1 = jnp.concatenate([w1, jnp.zeros((128 - C, E), F32)], axis=0)
        w1t_ref[...] = pltpu.bitcast(w1.T.astype(BF16), U32)
        for i in range(3):
            dwi = dw_ref[i].astype(F32)
            for j in range(3):
                dwb_ref[pl.ds((i * 3 + j) * C, C)] = jnp.broadcast_to(dwi[j:j + 1, :], (128, C)).T
        col = lax.broadcasted_iota(jnp.int32, (8, 128), 1) - lax.broadcasted_iota(jnp.int32, (8, 128), 0)
        for g in range(G):
            halves = []
            for ho in range(2):
                m = jnp.zeros((8, 128), F32)
                for i in range(3):
                    for j in range(3):
                        pair, r = divmod(ho + i, 2)
                        m = jnp.where(col == pair * 48 + j * 16 + r * 8, tap(i, j, g), m)
                halves.append(m)
            dwm_ref[g] = pltpu.bitcast(jnp.concatenate(halves, axis=0).astype(BF16), U32)

        def shift_stage(row, par, g):
            xc = pltpu.bitcast(xi_ref[pl.ds(row, 2), g].reshape(16, W), U32)
            sh_ref[par, g, 0] = shift(xc, True, jnp.uint32(0))
            sh_ref[par, g, 1] = xc
            sh_ref[par, g, 2] = shift(xc, False, jnp.uint32(0))

        def cv_row(par, g):
            return 8 * g + (C if (g < 2 and par) else 0)

        held = []

        def conv_stage(par, g):
            rhs = jnp.concatenate([sh_ref[p, g, j] for p in (par, 1 - par) for j in range(3)]
                                  + [jnp.zeros((16, W), U32)], axis=0)
            o = jnp.dot(pltpu.bitcast(dwm_ref[g], BF16), pltpu.bitcast(rhs, BF16),
                        preferred_element_type=F32)
            for ho in range(2):
                cv_ref[ho, pl.ds(cv_row(par, g), 8)] = o[8 * ho:8 * ho + 8]
            if g % 2 == 0:
                held.append(o)
                return
            p = held.pop()
            vs = (p + o, p * p + o * o)
            for ho in range(2):
                add_stats(st_ref.at[par], ho * NT, [v[8 * ho:8 * ho + 8] for v in vs], g == 1)

        def ln_stage(par, g):
            if g == 0:
                ln_stats(st_ref.at[par], rs_ref, 2 * NT)
            if g % 2 == 0:
                for ho in range(2):
                    v = ln_scale(cv_ref[ho, pl.ds(cv_row(par, g), 16)], rs_ref, ho * NT)
                    a_ref[par, ho, 4 * g:4 * g + 8] = pltpu.bitcast(v, U32)

        head.wait()
        for i in range(4):
            for g in range(G):
                if i == 3:
                    ln_stage(0, g)
                if i >= 2:
                    conv_stage(i % 2, g)
                shift_stage((NI - 1) * BS + 2 * i, i % 2, g)

        def body(b, _):
            in1(b).wait()

            @pl.when(b < NB - 1)
            def _():
                in1(b + 1).start()

            for s in range(BS // 2):
                par = s % 2
                row = (NI - 2 + b % 2) * BS + jnp.where(b == NB - 1, BS - 1, 2 * s)
                for g in range(G):
                    ho, e = divmod(g, G // 2)
                    lo, hi = e * 2 * E // G, (e + 1) * 2 * E // G
                    hid = mlp_in(pltpu.bitcast(a_ref[par, ho], BF16), lo, hi)
                    sq = acc_ref[lo:hi]
                    for t in range(NT):
                        sq = sq + tile(hid, t) * tile(hid, t)
                    acc_ref[lo:hi] = sq
                    if 2 * s + ho in KEEP:
                        h_ref[b, KEEP.index(2 * s + ho), lo:hi] = hid.astype(BF16)
                    ln_stage(1 - par, g)
                    conv_stage(par, g)
                    shift_stage(row, par, g)
            return 0

        lax.fori_loop(0, NB, body, 0, unroll=UNROLL1)
        in2(NI - 2).start()

        for cp in wts[2:]:
            cp.wait()
        ss = jnp.sum(acc_ref[...].T, axis=0, keepdims=True) * (1.0 / (4.0 * ALPHA * ALPHA))
        gx = jnp.sqrt(ss + 1e-6)
        nx = gx / (jnp.sum(gx, axis=1, keepdims=True) * (1.0 / E) + 1e-6)
        gam = gam_ref[...].astype(F32).reshape(1, E)
        bet = bet_ref[...].astype(F32).reshape(1, E)
        w2t = w2t_ref[...].astype(F32)
        scale = (gam * nx + 1.0) * (1.0 / (2.0 * ALPHA))
        w2s_ref[...] = pltpu.bitcast((w2t * scale).astype(BF16), U32)
        bias_ref[...] = jnp.broadcast_to(jnp.sum(w2t * bet, axis=1, keepdims=True), bias_ref.shape)

    pl.run_scoped(
        pass1,
        pltpu.VMEM((2, G, 3, 8, W), U32), pltpu.VMEM((2, C + 16, W), F32),
        pltpu.VMEM((2, 2, 16 * NT + 8, 128), F32), pltpu.VMEM((2 * NT, 8, 128), F32),
        pltpu.VMEM((2, 2, C // 2, W), U32), pltpu.VMEM((G, 8, 128), U32), pltpu.VMEM((E, 128), F32),
        *[pltpu.VMEM(r.shape, r.dtype) for r in (w1_hbm, w2t_hbm, dw_hbm, gam_hbm, bet_hbm)])

    def pass2(xf_ref, cv_ref, st_ref, rs_ref, a_ref, g_ref):
        def conv_piece(slot, n):
            u, g = divmod(n, G)
            c = pl.ds(8 * g, 8)
            rows = []
            for r in range(REC[u] - 1, REC[u] + 2):
                if u == 0 or r > REC[u]:
                    v = xi_ref[slot * BS + r, g].astype(F32)
                    if r in REC:
                        xf_ref[REC.index(r), c] = v
                else:
                    v = xf_ref[REC.index(r), c]
                rows.append(v)
            cols = []
            for j in range(3):
                p = [rows[i] * jnp.tile(tap(i, j, g), (1, NT)) for i in range(3)]
                cols.append((p[0] + p[1]) + p[2])
            o = shift(cols[0], True, 0.0) + cols[1] + shift(cols[2], False, 0.0)
            cv_ref[c] = o
            add_stats(st_ref, 0, (o, o * o), g == 0)
            if g == G - 1:
                ln_stats(st_ref, rs_ref, NT)
                a_ref[u] = ln_scale(cv_ref[...], rs_ref, 0)

        in2(0).wait()
        for n in range(len(REC) * G):
            conv_piece(0, n)

        def body(b, _):
            @pl.when(b + 1 < NB)
            def _():
                in2(b + 1).wait()

            @pl.when(b >= NO)
            def _():
                out2(b - NO).wait()

            @pl.when(b + NI - 1 < NB)
            def _():
                in2(b + NI - 1).start()

            nxt = jnp.minimum(b + 1, NB - 1) % NI
            spare = pl.ds(pl.multiple_of(9 * C + 8 * z_ref[0], 8), 8)
            done = []

            def issue(after, n):
                if n:
                    dwb_ref[spare] = after[-8:, -128:]
                for _ in range(n):
                    conv_piece(nxt, len(done))
                    done.append(0)

            for u in range(len(REC)):
                cnt = [int(n) for n in PIECES[u]]
                hid = mlp_in(a_ref[u], 0, E)
                g_ref[...] = hid.astype(BF16)
                for k in range(E // 128):
                    issue(hid[128 * k:128 * (k + 1)], cnt.pop(0))
                for r in KEPT_WITH[u] + (REC[u],):
                    for t2 in range(NT // 2):
                        ws = pl.ds(256 * t2, 256)
                        res = xi_ref[(b % NI) * BS + r, :, :, ws].astype(F32).reshape(C, 256)
                        o = []
                        for t in (2 * t2, 2 * t2 + 1):
                            ts = pl.ds(128 * t, 128)
                            hb = h_ref[b, KEEP.index(r), :, ts] if r in KEEP else g_ref[:, ts]
                            o.append(jnp.dot(pltpu.bitcast(w2s_ref[...], BF16), hb,
                                             preferred_element_type=F32) + bias_ref[...])
                            if t != 2:
                                issue(o[-1][:8], cnt.pop(0))
                        o = jnp.concatenate(o, axis=1) + res
                        xo_ref[b % NO, r, :, :, ws] = o.reshape(G, 8, 256).astype(BF16)
                    pltpu.make_async_copy(
                        xo_ref.at[b % NO, r], o_hbm.at[b * BS + r], sem_o.at[b % NO]).start()
                assert not cnt and len(done) < (u + 2) * G
            assert len(done) == len(REC) * G
            return 0

        lax.fori_loop(0, NB, body, 0, unroll=UNROLL2)
        for b in range(NB - NO, NB):
            out2(b).wait()

    pl.run_scoped(
        pass2,
        pltpu.VMEM((len(REC), C, W), F32), pltpu.VMEM((C, W), F32),
        pltpu.VMEM((2, 8 * NT + 8, 128), F32), pltpu.VMEM((NT, 8, 128), F32),
        pltpu.VMEM((len(REC), C, W), BF16), pltpu.VMEM((E, W), BF16))


@jax.jit
def pallas_standalone__modern_conv_block_convnext_v2__vision_kernel(x, dw, w1, w2, grn_gamma, grn_beta):
    B, H, W, C = x.shape
    E = w1.shape[1]
    G = C // 8
    assert (B, W, C, E) == (1, 512, 96, 384) and dw.shape == (3, 3, C) and H % (2 * BS) == 0
    xt = jnp.transpose(x, (0, 1, 3, 2)).reshape(H, G, 8, W)
    out = pl.pallas_call(
        functools.partial(_kernel, H=H, W=W, C=C, E=E),
        in_specs=[pl.BlockSpec(memory_space=pl.ANY)] * 6,
        out_specs=pl.BlockSpec(memory_space=pl.ANY),
        out_shape=jax.ShapeDtypeStruct((H, G, 8, W), x.dtype),
        scratch_shapes=[
            pltpu.VMEM((H // BS, len(KEEP), E, W), BF16),
            pltpu.VMEM((NI * BS + 1, G, 8, W), BF16),
            pltpu.VMEM((NO, BS, G, 8, W), BF16),
            pltpu.VMEM((9 * C + 8, 128), F32),
            pltpu.VMEM((E // 2, 128), U32),
            pltpu.VMEM((C // 2, E), U32),
            pltpu.VMEM((C, 128), F32),
            pltpu.SMEM((1,), jnp.int32),
            pltpu.SemaphoreType.DMA((NI,)),
            pltpu.SemaphoreType.DMA((NO,)),
            pltpu.SemaphoreType.DMA((5,)),
        ],
        compiler_params=pltpu.CompilerParams(
            vmem_limit_bytes=128 * 1024 * 1024,
            disable_bounds_checks=True,
            flags={"XLA_TPU_RESCHEDULE_DMA_DONES": True},
        ),
        name="convnext",
    )(xt, dw, w1, w2.T, grn_gamma, grn_beta)
    return jnp.transpose(out.reshape(B, H, C, W), (0, 1, 3, 2))
```

```python
import functools
import math

import jax
import jax.numpy as jnp
from jax import lax
import jax.experimental.pallas as pl
import jax.experimental.pallas.tpu as pltpu

F32 = jnp.float32
BF16 = jnp.bfloat16
U32 = jnp.uint32

_C0 = math.sqrt(2.0 / math.pi)
_C1 = 0.044715
ALPHA = (_C0 * _C1) ** (1.0 / 3.0)
K0 = _C0 / ALPHA

BS = 8
REC = (1, 2, 3)
KEEP = (0, 4, 5, 6, 7)
NI = 4
NO = 2
UNROLL1 = 8
UNROLL2 = 8
CF = 1
KEPT_WITH = ((4, 5), (6, 7), (0,))
PIECES = '100321120110-100321221211-011220110'.split('-')


def _kernel(x_hbm, dw_hbm, w1_hbm, w2t_hbm, gam_hbm, bet_hbm, o_hbm,
            h_ref, xi_ref, xo_ref, dwb_ref, w1t_ref, w2s_ref, bias_ref, z_ref,
            sem_i, sem_o, sem_w, *, H, W, C, E):
    NT = W // 128
    G = C // 8
    NB = H // BS

    def tile(v, t):
        return v[:, 128 * t:128 * (t + 1)]

    def tap(i, j, g):
        return dwb_ref[pl.ds((i * 3 + j) * C + 8 * g, 8)]

    def shift(v, right, zero):
        lane = lax.broadcasted_iota(jnp.int32, (v.shape[0], 128), 1)
        rl = [pltpu.roll(tile(v, t), 1 if right else 127, 1) for t in range(NT)]
        edge, step = (0, 1) if right else (127, -1)
        return jnp.concatenate(
            [jnp.where(lane == edge, rl[t - step] if 0 <= t - step < NT else zero, rl[t])
             for t in range(NT)], axis=1)

    def add_stats(st, q, vs, first):
        for k, v in enumerate(vs):
            for t in range(NT):
                r = pl.ds(8 * (q + t), 8)
                st[k, r] = tile(v, t) if first else st[k, r] + tile(v, t)

    def ln_stats(st, mr_ref, n):
        mom = []
        for k in range(2):
            v = [st[k, pl.ds(j, n, stride=8)] for j in range(8)]
            mom.append((((v[0] + v[1]) + (v[2] + v[3])) + ((v[4] + v[5]) + (v[6] + v[7]))) * (1.0 / C))
        var = jnp.maximum(mom[1] - mom[0] * mom[0], 0.0)
        r = lax.rsqrt(var + 1e-5) * ALPHA
        for q in range(n):
            mr_ref[0, q] = jnp.broadcast_to(mom[0][q:q + 1], (8, 128))
            mr_ref[1, q] = jnp.broadcast_to(r[q:q + 1], (8, 128))

    def ln_apply(v, mr_ref, q):
        m, r = (jnp.tile(jnp.concatenate([mr_ref[k, q + t] for t in range(NT)], axis=1),
                         (v.shape[0] // 8, 1)) for k in range(2))
        return (v - m) * r

    def mlp_in(a, lo, hi):
        a = jnp.concatenate([a, jnp.zeros((128 - C, W), BF16)], axis=0)
        y = jnp.dot(pltpu.bitcast(w1t_ref[lo // 2:hi // 2], BF16), a, preferred_element_type=F32)
        return (jnp.tanh((y * y + K0) * y) + 1.0) * y

    def load(row, n, slot, off=0):
        return pltpu.make_async_copy(
            x_hbm.at[pl.ds(row, n)], xi_ref.at[pl.ds(slot * BS + off, n)], sem_i.at[slot])

    def in1(b):
        return load(jnp.minimum(b * BS + BS - 1, H - BS), BS, NI - 2 + b % 2)

    def in2(b):
        return load(b * BS, BS, b % NI)

    def out2(b):
        return pltpu.make_async_copy(xo_ref.at[b % NO], o_hbm.at[pl.ds(b * BS, BS)], sem_o.at[b % NO])

    def pass1(sh_ref, cv_ref, st_ref, mr_ref, a_ref, dwm_ref, acc_ref,
              w1_ref, w2t_ref, dw_ref, gam_ref, bet_ref):
        wts = [pltpu.make_async_copy(src, dst, sem_w.at[k]) for k, (src, dst) in enumerate(
            zip((dw_hbm, w1_hbm, w2t_hbm, gam_hbm, bet_hbm), (dw_ref, w1_ref, w2t_ref, gam_ref, bet_ref)))]
        head = load(0, BS - 1, NI - 1, 1)
        wts[0].start()
        wts[1].start()
        head.start()
        in1(0).start()
        for cp in wts[2:]:
            cp.start()
        for b in range(NI - 2):
            in2(b).start()

        z_ref[0] = 0
        acc_ref[...] = jnp.zeros_like(acc_ref)
        xi_ref[(NI - 1) * BS] = jnp.zeros((G, 8, W), BF16)
        xi_ref[NI * BS] = jnp.zeros((G, 8, W), BF16)
        wts[0].wait()
        wts[1].wait()
        w1 = jnp.concatenate([w1_ref[...].astype(F32), jnp.zeros((128 - C, E), F32)], axis=0)
        w1t_ref[...] = pltpu.bitcast(w1.T.astype(BF16), U32)
        for i in range(3):
            dwi = dw_ref[i].astype(F32)
            for j in range(3):
                dwb_ref[pl.ds((i * 3 + j) * C, C)] = jnp.broadcast_to(dwi[j:j + 1, :], (128, C)).T
        col = lax.broadcasted_iota(jnp.int32, (8, 128), 1) - lax.broadcasted_iota(jnp.int32, (8, 128), 0)
        for g in range(G):
            halves = []
            for ho in range(2):
                m = jnp.zeros((8, 128), F32)
                for i in range(3):
                    for j in range(3):
                        pair, r = divmod(ho + i, 2)
                        m = jnp.where(col == pair * 48 + j * 16 + r * 8, tap(i, j, g), m)
                halves.append(m)
            dwm_ref[g] = pltpu.bitcast(jnp.concatenate(halves, axis=0).astype(BF16), U32)

        def shift_stage(row, par, g):
            xc = pltpu.bitcast(xi_ref[pl.ds(row, 2), g].reshape(16, W), U32)
            sh_ref[par, g, 0] = shift(xc, True, jnp.uint32(0))
            sh_ref[par, g, 1] = xc
            sh_ref[par, g, 2] = shift(xc, False, jnp.uint32(0))

        held = []

        def conv_stage(par, g):
            rhs = jnp.concatenate([sh_ref[p, g, j] for p in (par, 1 - par) for j in range(3)]
                                  + [jnp.zeros((16, W), U32)], axis=0)
            o = jnp.dot(pltpu.bitcast(dwm_ref[g], BF16), pltpu.bitcast(rhs, BF16),
                        preferred_element_type=F32)
            for ho in range(2):
                cv_ref[ho, pl.ds(8 * g, 8)] = o[8 * ho:8 * ho + 8]
            if g % 2 == 0:
                held.append(o)
                return
            p = held.pop()
            vs = (p + o, p * p + o * o)
            for ho in range(2):
                add_stats(st_ref, ho * NT, [v[8 * ho:8 * ho + 8] for v in vs], g == 1)

        def ln_stage(par, g, save=False):
            if g == 0:
                ln_stats(st_ref, mr_ref, 2 * NT)
            if g % 2 == 0:
                for ho in range(2):
                    v = ln_apply(cv_ref[ho, pl.ds(8 * g, 16)], mr_ref, ho * NT)
                    a_ref[par, ho, 4 * g:4 * g + 8] = pltpu.bitcast(v.astype(BF16), U32)
                    if save and 2 * par + ho in REC:
                        xo_ref[0, 2 * par + ho, g:g + 2] = v.reshape(2, 8, W).astype(BF16)

        head.wait()
        for i in range(4):
            for g in range(G):
                if i == 3:
                    ln_stage(0, g, True)
                if i >= 2:
                    conv_stage(i % 2, g)
                shift_stage((NI - 1) * BS + 2 * i, i % 2, g)
        for g in range(G):
            ln_stage(1, g, True)

        def body(b, _):
            in1(b).wait()

            @pl.when(b < NB - 1)
            def _():
                in1(b + 1).start()

            for s in range(BS // 2):
                par = s % 2
                row = (NI - 2 + b % 2) * BS + jnp.where(b == NB - 1, BS - 1, 2 * s)
                for g in range(G):
                    ho, e = divmod(g, G // 2)
                    lo, hi = e * 2 * E // G, (e + 1) * 2 * E // G
                    if CF:
                        ln_stage(1 - par, g)
                        conv_stage(par, g)
                    hid = mlp_in(pltpu.bitcast(a_ref[par, ho], BF16), lo, hi)
                    sq = acc_ref[lo:hi]
                    for t in range(NT):
                        sq = sq + tile(hid, t) * tile(hid, t)
                    acc_ref[lo:hi] = sq
                    if 2 * s + ho in KEEP:
                        h_ref[b, KEEP.index(2 * s + ho), lo:hi] = hid.astype(BF16)
                    if not CF:
                        ln_stage(1 - par, g)
                        conv_stage(par, g)
                    shift_stage(row, par, g)
            return 0

        lax.fori_loop(0, NB, body, 0, unroll=UNROLL1)
        in2(NI - 2).start()

        for cp in wts[2:]:
            cp.wait()
        ss = jnp.sum(acc_ref[...].T, axis=0, keepdims=True) * (1.0 / (4.0 * ALPHA * ALPHA))
        gx = jnp.sqrt(ss + 1e-6)
        nx = gx / (jnp.sum(gx, axis=1, keepdims=True) * (1.0 / E) + 1e-6)
        gam = gam_ref[...].astype(F32).reshape(1, E)
        bet = bet_ref[...].astype(F32).reshape(1, E)
        w2t = w2t_ref[...].astype(F32)
        scale = (gam * nx + 1.0) * (1.0 / (2.0 * ALPHA))
        w2s_ref[...] = pltpu.bitcast((w2t * scale).astype(BF16), U32)
        bias_ref[...] = jnp.broadcast_to(jnp.sum(w2t * bet, axis=1, keepdims=True), bias_ref.shape)

    pl.run_scoped(
        pass1,
        pltpu.VMEM((2, G, 3, 8, W), U32), pltpu.VMEM((2, C, W), F32),
        pltpu.VMEM((2, 16 * NT + 8, 128), F32), pltpu.VMEM((2, 2 * NT, 8, 128), F32),
        pltpu.VMEM((2, 2, C // 2, W), U32), pltpu.VMEM((G, 8, 128), U32), pltpu.VMEM((E, 128), F32),
        *[pltpu.VMEM(r.shape, r.dtype) for r in (w1_hbm, w2t_hbm, dw_hbm, gam_hbm, bet_hbm)])

    def pass2(xf_ref, cv_ref, st_ref, mr_ref, a_ref, g_ref):
        def conv_piece(slot, n):
            u, g = divmod(n, G)
            c = pl.ds(8 * g, 8)
            rows = []
            for r in range(REC[u] - 1, REC[u] + 2):
                if u == 0 or r > REC[u]:
                    v = xi_ref[slot * BS + r, g].astype(F32)
                    if r in REC:
                        xf_ref[REC.index(r), c] = v
                else:
                    v = xf_ref[REC.index(r), c]
                rows.append(v)
            cols = []
            for j in range(3):
                p = [rows[i] * jnp.tile(tap(i, j, g), (1, NT)) for i in range(3)]
                cols.append((p[0] + p[1]) + p[2])
            o = shift(cols[0], True, 0.0) + cols[1] + shift(cols[2], False, 0.0)
            cv_ref[c] = o
            add_stats(st_ref, 0, (o, o * o), g == 0)
            if g == G - 1:
                ln_stats(st_ref, mr_ref, NT)
                a_ref[u] = ln_apply(cv_ref[...], mr_ref, 0).astype(BF16)

        in2(0).wait()
        for u, r in enumerate(REC):
            a_ref[u] = xo_ref[0, r].reshape(C, W)

        def body(b, _):
            @pl.when(b + 1 < NB)
            def _():
                in2(b + 1).wait()

            @pl.when(b >= NO)
            def _():
                out2(b - NO).wait()

            @pl.when(b + NI - 1 < NB)
            def _():
                in2(b + NI - 1).start()

            nxt = jnp.minimum(b + 1, NB - 1) % NI
            spare = pl.ds(pl.multiple_of(9 * C + 8 * z_ref[0], 8), 8)
            done = []

            def issue(after, n):
                if n:
                    dwb_ref[spare] = after[-8:, -128:]
                for _ in range(n):
                    conv_piece(nxt, len(done))
                    done.append(0)

            for u in range(len(REC)):
                cnt = [int(n) for n in PIECES[u]]
                hid = mlp_in(a_ref[u], 0, E)
                g_ref[...] = hid.astype(BF16)
                for k in range(E // 128):
                    issue(hid[128 * k:128 * (k + 1)], cnt.pop(0))
                for r in KEPT_WITH[u] + (REC[u],):
                    for t2 in range(NT // 2):
                        ws = pl.ds(256 * t2, 256)
                        res = xi_ref[(b % NI) * BS + r, :, :, ws].astype(F32).reshape(C, 256)
                        o = []
                        for t in (2 * t2, 2 * t2 + 1):
                            ts = pl.ds(128 * t, 128)
                            hb = h_ref[b, KEEP.index(r), :, ts] if r in KEEP else g_ref[:, ts]
                            o.append(jnp.dot(pltpu.bitcast(w2s_ref[...], BF16), hb,
                                             preferred_element_type=F32) + bias_ref[...])
                            if t != 2:
                                issue(o[-1][:8], cnt.pop(0))
                        o = jnp.concatenate(o, axis=1) + res
                        xo_ref[b % NO, r, :, :, ws] = o.reshape(G, 8, 256).astype(BF16)
                    pltpu.make_async_copy(
                        xo_ref.at[b % NO, r], o_hbm.at[b * BS + r], sem_o.at[b % NO]).start()
                assert not cnt and len(done) < (u + 2) * G
            assert len(done) == len(REC) * G
            return 0

        lax.fori_loop(0, NB, body, 0, unroll=UNROLL2)
        for b in range(NB - NO, NB):
            out2(b).wait()

    pl.run_scoped(
        pass2,
        pltpu.VMEM((len(REC), C, W), F32), pltpu.VMEM((C, W), F32),
        pltpu.VMEM((2, 8 * NT + 8, 128), F32), pltpu.VMEM((2, NT, 8, 128), F32),
        pltpu.VMEM((len(REC), C, W), BF16), pltpu.VMEM((E, W), BF16))


@jax.jit
def pallas_standalone__modern_conv_block_convnext_v2__vision_kernel(x, dw, w1, w2, grn_gamma, grn_beta):
    B, H, W, C = x.shape
    E = w1.shape[1]
    G = C // 8
    assert (B, W, C, E) == (1, 512, 96, 384) and dw.shape == (3, 3, C) and H % (2 * BS) == 0
    xt = jnp.transpose(x, (0, 1, 3, 2)).reshape(H, G, 8, W)
    out = pl.pallas_call(
        functools.partial(_kernel, H=H, W=W, C=C, E=E),
        in_specs=[pl.BlockSpec(memory_space=pl.ANY)] * 6,
        out_specs=pl.BlockSpec(memory_space=pl.ANY),
        out_shape=jax.ShapeDtypeStruct((H, G, 8, W), x.dtype),
        scratch_shapes=[
            pltpu.VMEM((H // BS, len(KEEP), E, W), BF16),
            pltpu.VMEM((NI * BS + 1, G, 8, W), BF16),
            pltpu.VMEM((NO, BS, G, 8, W), BF16),
            pltpu.VMEM((9 * C + 8, 128), F32),
            pltpu.VMEM((E // 2, 128), U32),
            pltpu.VMEM((C // 2, E), U32),
            pltpu.VMEM((C, 128), F32),
            pltpu.SMEM((1,), jnp.int32),
            pltpu.SemaphoreType.DMA((NI,)),
            pltpu.SemaphoreType.DMA((NO,)),
            pltpu.SemaphoreType.DMA((5,)),
        ],
        compiler_params=pltpu.CompilerParams(
            vmem_limit_bytes=128 * 1024 * 1024,
            disable_bounds_checks=True,
            flags={"XLA_TPU_RESCHEDULE_DMA_DONES": True},
        ),
        name="convnext",
    )(xt, dw, w1, w2.T, grn_gamma, grn_beta)
    return jnp.transpose(out.reshape(B, H, C, W), (0, 1, 3, 2))
```

```python
import functools
import math

import jax
import jax.numpy as jnp
from jax import lax
import jax.experimental.pallas as pl
import jax.experimental.pallas.tpu as pltpu

F32 = jnp.float32
BF16 = jnp.bfloat16
U32 = jnp.uint32

_C0 = math.sqrt(2.0 / math.pi)
_C1 = 0.044715
ALPHA = (_C0 * _C1) ** (1.0 / 3.0)
K0 = _C0 / ALPHA

BS = 8
REC = (1, 2, 3)
KEEP = (0, 4, 5, 6, 7)
NI = 4
NO = 2
UNROLL1 = 8
UNROLL2 = 8
KEPT_WITH = ((4, 5), (6, 7), (0,))
PIECES = ('100321120210', '001221221311', '001210210')


def _kernel(x_hbm, dw_hbm, w1_hbm, w2t_hbm, gam_hbm, bet_hbm, o_hbm,
            h_ref, xi_ref, xo_ref, dwb_ref, w1t_ref, w2s_ref, bias_ref, z_ref,
            sem_i, sem_o, sem_w, *, H, W, C, E):
    NT = W // 128
    G = C // 8
    NB = H // BS

    def tile(v, t):
        return v[:, 128 * t:128 * (t + 1)]

    def tap(i, j, g):
        return dwb_ref[pl.ds((i * 3 + j) * C + 8 * g, 8)]

    def shift(v, right, zero):
        lane = lax.broadcasted_iota(jnp.int32, (v.shape[0], 128), 1)
        rl = [pltpu.roll(tile(v, t), 1 if right else 127, 1) for t in range(NT)]
        edge, step = (0, 1) if right else (127, -1)
        return jnp.concatenate(
            [jnp.where(lane == edge, rl[t - step] if 0 <= t - step < NT else zero, rl[t])
             for t in range(NT)], axis=1)

    def add_stats(st, q, vs, first):
        for k, v in enumerate(vs):
            for t in range(NT):
                r = pl.ds(8 * (q + t), 8)
                st[k, r] = tile(v, t) if first else st[k, r] + tile(v, t)

    def ln_stats(st, mr_ref, n):
        mom = []
        for k in range(2):
            v = [st[k, pl.ds(j, n, stride=8)] for j in range(8)]
            mom.append((((v[0] + v[1]) + (v[2] + v[3])) + ((v[4] + v[5]) + (v[6] + v[7]))) * (1.0 / C))
        var = jnp.maximum(mom[1] - mom[0] * mom[0], 0.0)
        r = lax.rsqrt(var + 1e-5) * ALPHA
        for q in range(n):
            mr_ref[0, q] = jnp.broadcast_to(mom[0][q:q + 1], (8, 128))
            mr_ref[1, q] = jnp.broadcast_to(r[q:q + 1], (8, 128))

    def ln_apply(v, mr_ref, q):
        m, r = (jnp.tile(jnp.concatenate([mr_ref[k, q + t] for t in range(NT)], axis=1),
                         (v.shape[0] // 8, 1)) for k in range(2))
        return (v - m) * r

    def mlp_in(a, lo, hi):
        a = jnp.concatenate([a, jnp.zeros((128 - C, W), BF16)], axis=0)
        y = jnp.dot(pltpu.bitcast(w1t_ref[lo // 2:hi // 2], BF16), a, preferred_element_type=F32)
        return (jnp.tanh((y * y + K0) * y) + 1.0) * y

    def load(row, n, slot, off=0):
        return pltpu.make_async_copy(
            x_hbm.at[pl.ds(row, n)], xi_ref.at[pl.ds(slot * BS + off, n)], sem_i.at[slot])

    def in1(b):
        return load(jnp.minimum(b * BS + BS - 1, H - BS), BS, NI - 2 + b % 2)

    def in2(b):
        return load(b * BS, BS, b % NI)

    def out2(b):
        return pltpu.make_async_copy(xo_ref.at[b % NO], o_hbm.at[pl.ds(b * BS, BS)], sem_o.at[b % NO])

    def pass1(sh_ref, cv_ref, st_ref, mr_ref, a_ref, dwm_ref, acc_ref,
              w1_ref, w2t_ref, dw_ref, gam_ref, bet_ref):
        wts = [pltpu.make_async_copy(src, dst, sem_w.at[k]) for k, (src, dst) in enumerate(
            zip((dw_hbm, w1_hbm, w2t_hbm, gam_hbm, bet_hbm), (dw_ref, w1_ref, w2t_ref, gam_ref, bet_ref)))]
        head = load(0, BS - 1, NI - 1, 1)
        wts[0].start()
        wts[1].start()
        head.start()
        in1(0).start()
        for cp in wts[2:]:
            cp.start()
        for b in range(NI - 2):
            in2(b).start()

        z_ref[0] = 0
        acc_ref[...] = jnp.zeros_like(acc_ref)
        xi_ref[(NI - 1) * BS] = jnp.zeros((G, 8, W), BF16)
        xi_ref[NI * BS] = jnp.zeros((G, 8, W), BF16)
        wts[0].wait()
        wts[1].wait()
        w1 = jnp.concatenate([w1_ref[...].astype(F32), jnp.zeros((128 - C, E), F32)], axis=0)
        w1t_ref[...] = pltpu.bitcast(w1.T.astype(BF16), U32)
        for i in range(3):
            dwi = dw_ref[i].astype(F32)
            for j in range(3):
                dwb_ref[pl.ds((i * 3 + j) * C, C)] = jnp.broadcast_to(dwi[j:j + 1, :], (128, C)).T
        col = lax.broadcasted_iota(jnp.int32, (8, 128), 1) - lax.broadcasted_iota(jnp.int32, (8, 128), 0)
        for g in range(G):
            halves = []
            for ho in range(2):
                m = jnp.zeros((8, 128), F32)
                for i in range(3):
                    for j in range(3):
                        pair, r = divmod(ho + i, 2)
                        m = jnp.where(col == pair * 48 + j * 16 + r * 8, tap(i, j, g), m)
                halves.append(m)
            dwm_ref[g] = pltpu.bitcast(jnp.concatenate(halves, axis=0).astype(BF16), U32)

        def shift_stage(row, par, g):
            xc = pltpu.bitcast(xi_ref[pl.ds(row, 2), g].reshape(16, W), U32)
            sh_ref[par, g, 0] = shift(xc, True, jnp.uint32(0))
            sh_ref[par, g, 1] = xc
            sh_ref[par, g, 2] = shift(xc, False, jnp.uint32(0))

        held = []

        def conv_stage(par, g):
            rhs = jnp.concatenate([sh_ref[p, g, j] for p in (par, 1 - par) for j in range(3)]
                                  + [jnp.zeros((16, W), U32)], axis=0)
            o = jnp.dot(pltpu.bitcast(dwm_ref[g], BF16), pltpu.bitcast(rhs, BF16),
                        preferred_element_type=F32)
            for ho in range(2):
                cv_ref[ho, pl.ds(8 * g, 8)] = o[8 * ho:8 * ho + 8]
            if g % 2 == 0:
                held.append(o)
                return
            p = held.pop()
            vs = (p + o, p * p + o * o)
            for ho in range(2):
                add_stats(st_ref, ho * NT, [v[8 * ho:8 * ho + 8] for v in vs], g == 1)

        def ln_stage(par, g, save=False):
            if g == 0:
                ln_stats(st_ref, mr_ref, 2 * NT)
            if g % 2 == 0:
                for ho in range(2):
                    v = ln_apply(cv_ref[ho, pl.ds(8 * g, 16)], mr_ref, ho * NT)
                    a_ref[par, ho, 4 * g:4 * g + 8] = pltpu.bitcast(v.astype(BF16), U32)
                    if save and 2 * par + ho in REC:
                        xo_ref[0, 2 * par + ho, g:g + 2] = v.reshape(2, 8, W).astype(BF16)

        head.wait()
        for i in range(4):
            for g in range(G):
                if i == 3:
                    ln_stage(0, g, True)
                if i >= 2:
                    conv_stage(i % 2, g)
                shift_stage((NI - 1) * BS + 2 * i, i % 2, g)
        for g in range(G):
            ln_stage(1, g, True)

        def body(b, _):
            in1(b).wait()

            @pl.when(b < NB - 1)
            def _():
                in1(b + 1).start()

            for s in range(BS // 2):
                par = s % 2
                row = (NI - 2 + b % 2) * BS + jnp.where(b == NB - 1, BS - 1, 2 * s)
                for g in range(G):
                    ho, e = divmod(g, G // 2)
                    lo, hi = e * 2 * E // G, (e + 1) * 2 * E // G
                    ln_stage(1 - par, g)
                    conv_stage(par, g)
                    hid = mlp_in(pltpu.bitcast(a_ref[par, ho], BF16), lo, hi)
                    sq = acc_ref[lo:hi]
                    for t in (2, 3, 0, 1):
                        sq = sq + tile(hid, t) * tile(hid, t)
                    acc_ref[lo:hi] = sq
                    if 2 * s + ho in KEEP:
                        h_ref[b, KEEP.index(2 * s + ho), lo:hi] = hid.astype(BF16)
                    shift_stage(row, par, g)
            return 0

        lax.fori_loop(0, NB, body, 0, unroll=UNROLL1)
        in2(NI - 2).start()

        for cp in wts[2:]:
            cp.wait()
        ss = jnp.sum(acc_ref[...].T, axis=0, keepdims=True) * (1.0 / (4.0 * ALPHA * ALPHA))
        gx = jnp.sqrt(ss + 1e-6)
        nx = gx / (jnp.sum(gx, axis=1, keepdims=True) * (1.0 / E) + 1e-6)
        gam = gam_ref[...].astype(F32).reshape(1, E)
        bet = bet_ref[...].astype(F32).reshape(1, E)
        w2t = w2t_ref[...].astype(F32)
        scale = (gam * nx + 1.0) * (1.0 / (2.0 * ALPHA))
        w2s_ref[...] = pltpu.bitcast((w2t * scale).astype(BF16), U32)
        bias_ref[...] = jnp.broadcast_to(jnp.sum(w2t * bet, axis=1, keepdims=True), bias_ref.shape)

    pl.run_scoped(
        pass1,
        pltpu.VMEM((2, G, 3, 8, W), U32), pltpu.VMEM((2, C, W), F32),
        pltpu.VMEM((2, 16 * NT + 8, 128), F32), pltpu.VMEM((2, 2 * NT, 8, 128), F32),
        pltpu.VMEM((2, 2, C // 2, W), U32), pltpu.VMEM((G, 8, 128), U32), pltpu.VMEM((E, 128), F32),
        *[pltpu.VMEM(r.shape, r.dtype) for r in (w1_hbm, w2t_hbm, dw_hbm, gam_hbm, bet_hbm)])

    def pass2(xf_ref, cv_ref, st_ref, mr_ref, a_ref, g_ref):
        def conv_piece(slot, n):
            u, g = divmod(n, G)
            c = pl.ds(8 * g, 8)
            rows = []
            for r in range(REC[u] - 1, REC[u] + 2):
                if u == 0 or r > REC[u]:
                    v = xi_ref[slot * BS + r, g].astype(F32)
                    if r in REC:
                        xf_ref[REC.index(r), c] = v
                else:
                    v = xf_ref[REC.index(r), c]
                rows.append(v)
            cols = []
            for j in range(3):
                p = [rows[i] * jnp.tile(tap(i, j, g), (1, NT)) for i in range(3)]
                cols.append((p[0] + p[1]) + p[2])
            o = shift(cols[0], True, 0.0) + cols[1] + shift(cols[2], False, 0.0)
            cv_ref[c] = o
            add_stats(st_ref, 0, (o, o * o), g == 0)
            if g == G - 1:
                ln_stats(st_ref, mr_ref, NT)
                a_ref[u] = ln_apply(cv_ref[...], mr_ref, 0).astype(BF16)

        in2(0).wait()
        for u, r in enumerate(REC):
            a_ref[u] = xo_ref[0, r].reshape(C, W)

        def body(b, _):
            @pl.when(b + 1 < NB)
            def _():
                in2(b + 1).wait()

            @pl.when(b >= NO)
            def _():
                out2(b - NO).wait()

            @pl.when(b + NI - 1 < NB)
            def _():
                in2(b + NI - 1).start()

            nxt = jnp.minimum(b + 1, NB - 1) % NI
            spare = pl.ds(pl.multiple_of(9 * C + 8 * z_ref[0], 8), 8)
            done = []

            def issue(after, n):
                if n:
                    dwb_ref[spare] = after[-8:, -128:]
                for _ in range(n):
                    conv_piece(nxt, len(done))
                    done.append(0)

            for u in range(len(REC)):
                cnt = [int(n) for n in PIECES[u]]
                hid = mlp_in(a_ref[u], 0, E)
                g_ref[...] = hid.astype(BF16)
                for k in range(E // 128):
                    issue(hid[128 * k:128 * (k + 1)], cnt.pop(0))
                for r in KEPT_WITH[u] + (REC[u],):
                    for t2 in range(NT // 2):
                        ws = pl.ds(256 * t2, 256)
                        res = xi_ref[(b % NI) * BS + r, :, :, ws].astype(F32).reshape(C, 256)
                        o = []
                        for t in (2 * t2, 2 * t2 + 1):
                            ts = pl.ds(128 * t, 128)
                            hb = h_ref[b, KEEP.index(r), :, ts] if r in KEEP else g_ref[:, ts]
                            o.append(jnp.dot(pltpu.bitcast(w2s_ref[...], BF16), hb,
                                             preferred_element_type=F32) + bias_ref[...])
                            if t != 2:
                                issue(o[-1][:8], cnt.pop(0))
                        o = jnp.concatenate(o, axis=1) + res
                        xo_ref[b % NO, r, :, :, ws] = o.reshape(G, 8, 256).astype(BF16)
                    pltpu.make_async_copy(
                        xo_ref.at[b % NO, r], o_hbm.at[b * BS + r], sem_o.at[b % NO]).start()
                assert not cnt and len(done) < (u + 2) * G
            assert len(done) == len(REC) * G
            return 0

        lax.fori_loop(0, NB, body, 0, unroll=UNROLL2)
        for b in range(NB - NO, NB):
            out2(b).wait()

    pl.run_scoped(
        pass2,
        pltpu.VMEM((len(REC), C, W), F32), pltpu.VMEM((C, W), F32),
        pltpu.VMEM((2, 8 * NT + 8, 128), F32), pltpu.VMEM((2, NT, 8, 128), F32),
        pltpu.VMEM((len(REC), C, W), BF16), pltpu.VMEM((E, W), BF16))


@jax.jit
def pallas_standalone__modern_conv_block_convnext_v2__vision_kernel(x, dw, w1, w2, grn_gamma, grn_beta):
    B, H, W, C = x.shape
    E = w1.shape[1]
    G = C // 8
    assert (B, W, C, E) == (1, 512, 96, 384) and dw.shape == (3, 3, C) and H % (2 * BS) == 0
    xt = jnp.transpose(x, (0, 1, 3, 2)).reshape(H, G, 8, W)
    out = pl.pallas_call(
        functools.partial(_kernel, H=H, W=W, C=C, E=E),
        in_specs=[pl.BlockSpec(memory_space=pl.ANY)] * 6,
        out_specs=pl.BlockSpec(memory_space=pl.ANY),
        out_shape=jax.ShapeDtypeStruct((H, G, 8, W), x.dtype),
        scratch_shapes=[
            pltpu.VMEM((H // BS, len(KEEP), E, W), BF16),
            pltpu.VMEM((NI * BS + 1, G, 8, W), BF16),
            pltpu.VMEM((NO, BS, G, 8, W), BF16),
            pltpu.VMEM((9 * C + 8, 128), F32),
            pltpu.VMEM((E // 2, 128), U32),
            pltpu.VMEM((C // 2, E), U32),
            pltpu.VMEM((C, 128), F32),
            pltpu.SMEM((1,), jnp.int32),
            pltpu.SemaphoreType.DMA((NI,)),
            pltpu.SemaphoreType.DMA((NO,)),
            pltpu.SemaphoreType.DMA((5,)),
        ],
        compiler_params=pltpu.CompilerParams(
            vmem_limit_bytes=128 * 1024 * 1024,
            disable_bounds_checks=True,
            flags={"XLA_TPU_RESCHEDULE_DMA_DONES": True},
        ),
        name="convnext",
    )(xt, dw, w1, w2.T, grn_gamma, grn_beta)
    return jnp.transpose(out.reshape(B, H, C, W), (0, 1, 3, 2))
```

```python
import functools
import math

import jax
import jax.numpy as jnp
from jax import lax
import jax.experimental.pallas as pl
import jax.experimental.pallas.tpu as pltpu

F32 = jnp.float32
BF16 = jnp.bfloat16
U32 = jnp.uint32

_C0 = math.sqrt(2.0 / math.pi)
_C1 = 0.044715
ALPHA = (_C0 * _C1) ** (1.0 / 3.0)
K0 = _C0 / ALPHA

BS = 8
REC = (1, 2, 3)
KEEP = (0, 4, 5, 6, 7)
NI = 4
NO = 2
UNROLL1 = 8
UNROLL2 = 8
KEPT_WITH = ((4, 5), (6, 7), (0,))
PIECES = ('100321120210', '001221230212', '100210210')


def _kernel(x_hbm, dw_hbm, w1_hbm, w2t_hbm, gam_hbm, bet_hbm, o_hbm,
            h_ref, xi_ref, xo_ref, dwb_ref, w1t_ref, w2s_ref, bias_ref, z_ref,
            sem_i, sem_o, sem_w, *, H, W, C, E):
    NT = W // 128
    G = C // 8
    NB = H // BS

    def tile(v, t):
        return v[:, 128 * t:128 * (t + 1)]

    def tap(i, j, g):
        return dwb_ref[pl.ds((i * 3 + j) * C + 8 * g, 8)]

    def shift(v, right, zero):
        lane = lax.broadcasted_iota(jnp.int32, (v.shape[0], 128), 1)
        rl = [pltpu.roll(tile(v, t), 1 if right else 127, 1) for t in range(NT)]
        edge, step = (0, 1) if right else (127, -1)
        return jnp.concatenate(
            [jnp.where(lane == edge, rl[t - step] if 0 <= t - step < NT else zero, rl[t])
             for t in range(NT)], axis=1)

    def add_part(st, q, v, first):
        for t in range(NT):
            r = pl.ds(8 * (q + t), 8)
            st[r] = tile(v, t) if first else st[r] + tile(v, t)

    def channel_mean(st, n):
        v = [st[pl.ds(j, n, stride=8)] for j in range(8)]
        return (((v[0] + v[1]) + (v[2] + v[3])) + ((v[4] + v[5]) + (v[6] + v[7]))) * (1.0 / C)

    def rstd(st, n):
        return lax.rsqrt(channel_mean(st, n) + 1e-5) * ALPHA

    def spread(bc, v):
        for q in range(v.shape[0]):
            bc[q] = jnp.broadcast_to(v[q:q + 1], (8, 128))

    def per_pixel(bc, q, rows):
        return jnp.tile(jnp.concatenate([bc[q + t] for t in range(NT)], axis=1), (rows // 8, 1))

    def spread_taps(dw_ref):
        for i in range(3):
            dwi = dw_ref[i].astype(F32)
            for j in range(3):
                dwb_ref[pl.ds((i * 3 + j) * C, C)] = jnp.broadcast_to(dwi[j:j + 1, :], (128, C)).T

    def mlp_in(a, lo, hi):
        a = jnp.concatenate([a, jnp.zeros((128 - C, W), BF16)], axis=0)
        y = jnp.dot(pltpu.bitcast(w1t_ref[lo // 2:hi // 2], BF16), a, preferred_element_type=F32)
        return (jnp.tanh((y * y + K0) * y) + 1.0) * y

    def load(row, n, slot, off=0):
        return pltpu.make_async_copy(
            x_hbm.at[pl.ds(row, n)], xi_ref.at[pl.ds(slot * BS + off, n)], sem_i.at[slot])

    def in1(b):
        return load(jnp.minimum(b * BS + BS + 1, H - BS), BS, NI - 1 - b % 2)

    def in2(b):
        return load(b * BS, BS, b % NI)

    def out2(b):
        return pltpu.make_async_copy(xo_ref.at[b % NO], o_hbm.at[pl.ds(b * BS, BS)], sem_o.at[b % NO])

    def pass1(sh_ref, cv_ref, st_ref, mr_ref, a_ref, dwm_ref, acc_ref,
              w1_ref, w2t_ref, dw_ref, gam_ref, bet_ref):
        wts = [pltpu.make_async_copy(src, dst, sem_w.at[k]) for k, (src, dst) in enumerate(
            zip((dw_hbm, w1_hbm, w2t_hbm, gam_hbm, bet_hbm), (dw_ref, w1_ref, w2t_ref, gam_ref, bet_ref)))]
        head = load(0, BS + 1, 0, 1)
        wts[0].start()
        wts[1].start()
        head.start()
        in1(0).start()
        for cp in wts[2:]:
            cp.start()

        z_ref[0] = 0
        acc_ref[...] = jnp.zeros_like(acc_ref)
        xi_ref[0] = jnp.zeros((G, 8, W), BF16)
        xi_ref[NI * BS] = jnp.zeros((G, 8, W), BF16)
        wts[0].wait()
        wts[1].wait()
        w1 = jnp.concatenate([w1_ref[...].astype(F32), jnp.zeros((128 - C, E), F32)], axis=0)
        w1t_ref[...] = pltpu.bitcast(w1.T.astype(BF16), U32)
        spread_taps(dw_ref)
        col = lax.broadcasted_iota(jnp.int32, (8, 128), 1) - lax.broadcasted_iota(jnp.int32, (8, 128), 0)
        for g in range(G):
            halves = []
            for ho in range(2):
                m = jnp.zeros((8, 128), F32)
                for i in range(3):
                    for j in range(3):
                        pair, r = divmod(ho + i, 2)
                        m = jnp.where(col == pair * 48 + j * 16 + r * 8, tap(i, j, g), m)
                halves.append(m)
            dwm_ref[g] = pltpu.bitcast(jnp.concatenate(halves, axis=0).astype(BF16), U32)

        def shift_stage(row, par, g):
            xc = pltpu.bitcast(xi_ref[pl.ds(row, 2), g].reshape(16, W), U32)
            sh_ref[par, g, 0] = shift(xc, True, jnp.uint32(0))
            sh_ref[par, g, 1] = xc
            sh_ref[par, g, 2] = shift(xc, False, jnp.uint32(0))

        held = []

        def conv_stage(par, g):
            rhs = jnp.concatenate([sh_ref[p, g, j] for p in (par, 1 - par) for j in range(3)]
                                  + [jnp.zeros((16, W), U32)], axis=0)
            o = jnp.dot(pltpu.bitcast(dwm_ref[g], BF16), pltpu.bitcast(rhs, BF16),
                        preferred_element_type=F32)
            for ho in range(2):
                cv_ref[ho, pl.ds(8 * g, 8)] = o[8 * ho:8 * ho + 8]
            if g % 2 == 0:
                held.append(o)
                return
            o = held.pop() + o
            for ho in range(2):
                add_part(st_ref.at[0], ho * NT, o[8 * ho:8 * ho + 8], g == 1)

        def dev(ho, t, g):
            return pl.ds((ho * NT + t) * C + 8 * g, 16)

        def var_stage(g):
            if g == 0:
                spread(mr_ref.at[0], channel_mean(st_ref.at[0], 2 * NT))
            if g % 2 == 0:
                for ho in range(2):
                    d = cv_ref[ho, pl.ds(8 * g, 16)] - per_pixel(mr_ref.at[0], ho * NT, 16)
                    for t in range(NT):
                        dwb_ref[dev(ho, t, g)] = tile(d, t)
                    d = d * d
                    add_part(st_ref.at[1], ho * NT, d[:8] + d[8:], g == 0)

        def norm_stage(par, g, save=False):
            if g == 0:
                spread(mr_ref.at[1], rstd(st_ref.at[1], 2 * NT))
            if g % 2 == 0:
                for ho in range(2):
                    d = jnp.concatenate([dwb_ref[dev(ho, t, g)] for t in range(NT)], axis=1)
                    v = d * per_pixel(mr_ref.at[1], ho * NT, 16)
                    a_ref[par, ho, 4 * g:4 * g + 8] = pltpu.bitcast(v.astype(BF16), U32)
                    if save and 2 * par + ho in REC:
                        xo_ref[0, 2 * par + ho, g:g + 2] = v.reshape(2, 8, W).astype(BF16)

        head.wait()
        for i in range(5):
            for g in range(G):
                if i >= 4:
                    norm_stage(0, g, True)
                if i >= 3:
                    var_stage(g)
                if i >= 2:
                    conv_stage(i % 2, g)
                shift_stage(2 * i, i % 2, g)
        for g in range(G):
            norm_stage(1, g, True)
        for b in range(NI - 2):
            in2(b).start()

        def body(b, _):
            in1(b).wait()

            @pl.when(b < NB - 1)
            def _():
                in1(b + 1).start()

            for s in range(BS // 2):
                par = s % 2
                row = (NI - 1 - b % 2) * BS + jnp.where(b == NB - 2, 2 * s + 1, 2 * s)
                for g in range(G):
                    ho, e = divmod(g, G // 2)
                    lo, hi = e * 2 * E // G, (e + 1) * 2 * E // G
                    norm_stage(1 - par, g)
                    var_stage(g)
                    conv_stage(1 - par, g)
                    hid = mlp_in(pltpu.bitcast(a_ref[par, ho], BF16), lo, hi)
                    sq = acc_ref[lo:hi]
                    for t in (1, 0, 2, 3):
                        sq = sq + tile(hid, t) * tile(hid, t)
                    acc_ref[lo:hi] = sq
                    if 2 * s + ho in KEEP:
                        h_ref[b, KEEP.index(2 * s + ho), lo:hi] = hid.astype(BF16)
                    shift_stage(row, 1 - par, g)
            return 0

        lax.fori_loop(0, NB, body, 0, unroll=UNROLL1)
        in2(NI - 2).start()

        spread_taps(dw_ref)
        for cp in wts[2:]:
            cp.wait()
        ss = jnp.sum(acc_ref[...].T, axis=0, keepdims=True) * (1.0 / (4.0 * ALPHA * ALPHA))
        gx = jnp.sqrt(ss + 1e-6)
        nx = gx / (jnp.sum(gx, axis=1, keepdims=True) * (1.0 / E) + 1e-6)
        gam = gam_ref[...].astype(F32).reshape(1, E)
        bet = bet_ref[...].astype(F32).reshape(1, E)
        w2t = w2t_ref[...].astype(F32)
        scale = (gam * nx + 1.0) * (1.0 / (2.0 * ALPHA))
        w2s_ref[...] = pltpu.bitcast((w2t * scale).astype(BF16), U32)
        bias_ref[...] = jnp.broadcast_to(jnp.sum(w2t * bet, axis=1, keepdims=True), bias_ref.shape)

    pl.run_scoped(
        pass1,
        pltpu.VMEM((2, G, 3, 8, W), U32), pltpu.VMEM((2, C, W), F32),
        pltpu.VMEM((2, 16 * NT + 8, 128), F32), pltpu.VMEM((2, 2 * NT, 8, 128), F32),
        pltpu.VMEM((2, 2, C // 2, W), U32), pltpu.VMEM((G, 8, 128), U32), pltpu.VMEM((E, 128), F32),
        *[pltpu.VMEM(r.shape, r.dtype) for r in (w1_hbm, w2t_hbm, dw_hbm, gam_hbm, bet_hbm)])

    def pass2(xf_ref, cv_ref, dv_ref, st_ref, mr_ref, a_ref, g_ref):
        def conv_piece(slot, n):
            u, g = divmod(n, G)
            c = pl.ds(8 * g, 8)
            rows = []
            for r in range(REC[u] - 1, REC[u] + 2):
                if u == 0 or r > REC[u]:
                    v = xi_ref[slot * BS + r, g].astype(F32)
                    if r in REC:
                        xf_ref[REC.index(r), c] = v
                else:
                    v = xf_ref[REC.index(r), c]
                rows.append(v)
            cols = []
            for j in range(3):
                p = [rows[i] * jnp.tile(tap(i, j, g), (1, NT)) for i in range(3)]
                cols.append((p[0] + p[1]) + p[2])
            o = shift(cols[0], True, 0.0) + cols[1] + shift(cols[2], False, 0.0)
            cv_ref[c] = o
            add_part(st_ref.at[0], 0, o, g == 0)
            if g == G - 1:
                spread(mr_ref.at[0], channel_mean(st_ref.at[0], NT))
                sq = None
                for k in range(G):
                    d = cv_ref[pl.ds(8 * k, 8)] - per_pixel(mr_ref.at[0], 0, 8)
                    dv_ref[pl.ds(8 * k, 8)] = d
                    sq = d * d if sq is None else sq + d * d
                add_part(st_ref.at[1], 0, sq, True)
                spread(mr_ref.at[1], rstd(st_ref.at[1], NT))
                a_ref[u] = (dv_ref[...] * per_pixel(mr_ref.at[1], 0, C)).astype(BF16)

        in2(0).wait()
        for u, r in enumerate(REC):
            a_ref[u] = xo_ref[0, r].reshape(C, W)

        def body(b, _):
            @pl.when(b + 1 < NB)
            def _():
                in2(b + 1).wait()

            @pl.when(b >= NO)
            def _():
                out2(b - NO).wait()

            @pl.when(b + NI - 1 < NB)
            def _():
                in2(b + NI - 1).start()

            nxt = jnp.minimum(b + 1, NB - 1) % NI
            spare = pl.ds(pl.multiple_of(9 * C + 8 * z_ref[0], 8), 8)
            done = []

            def issue(after, n):
                if n:
                    dwb_ref[spare] = after[-8:, -128:]
                for _ in range(n):
                    conv_piece(nxt, len(done))
                    done.append(0)

            for u in range(len(REC)):
                cnt = [int(n) for n in PIECES[u]]
                hid = mlp_in(a_ref[u], 0, E)
                g_ref[...] = hid.astype(BF16)
                for k in range(E // 128):
                    issue(hid[128 * k:128 * (k + 1)], cnt.pop(0))
                for r in KEPT_WITH[u] + (REC[u],):
                    for t2 in range(NT // 2):
                        ws = pl.ds(256 * t2, 256)
                        res = xi_ref[(b % NI) * BS + r, :, :, ws].astype(F32).reshape(C, 256)
                        o = []
                        for t in (2 * t2, 2 * t2 + 1):
                            ts = pl.ds(128 * t, 128)
                            hb = h_ref[b, KEEP.index(r), :, ts] if r in KEEP else g_ref[:, ts]
                            o.append(jnp.dot(pltpu.bitcast(w2s_ref[...], BF16), hb,
                                             preferred_element_type=F32) + bias_ref[...])
                            if t != 2:
                                issue(o[-1][:8], cnt.pop(0))
                        o = jnp.concatenate(o, axis=1) + res
                        xo_ref[b % NO, r, :, :, ws] = o.reshape(G, 8, 256).astype(BF16)
                    pltpu.make_async_copy(
                        xo_ref.at[b % NO, r], o_hbm.at[b * BS + r], sem_o.at[b % NO]).start()
                assert not cnt and len(done) < (u + 2) * G
            assert len(done) == len(REC) * G
            return 0

        lax.fori_loop(0, NB, body, 0, unroll=UNROLL2)
        for b in range(NB - NO, NB):
            out2(b).wait()

    pl.run_scoped(
        pass2,
        pltpu.VMEM((len(REC), C, W), F32), pltpu.VMEM((C, W), F32), pltpu.VMEM((C, W), F32),
        pltpu.VMEM((2, 8 * NT + 8, 128), F32), pltpu.VMEM((2, NT, 8, 128), F32),
        pltpu.VMEM((len(REC), C, W), BF16), pltpu.VMEM((E, W), BF16))


@jax.jit
def pallas_standalone__modern_conv_block_convnext_v2__vision_kernel(x, dw, w1, w2, grn_gamma, grn_beta):
    B, H, W, C = x.shape
    E = w1.shape[1]
    G = C // 8
    assert (B, W, C, E) == (1, 512, 96, 384) and dw.shape == (3, 3, C) and H % (2 * BS) == 0
    xt = jnp.transpose(x, (0, 1, 3, 2)).reshape(H, G, 8, W)
    out = pl.pallas_call(
        functools.partial(_kernel, H=H, W=W, C=C, E=E),
        in_specs=[pl.BlockSpec(memory_space=pl.ANY)] * 6,
        out_specs=pl.BlockSpec(memory_space=pl.ANY),
        out_shape=jax.ShapeDtypeStruct((H, G, 8, W), x.dtype),
        scratch_shapes=[
            pltpu.VMEM((H // BS, len(KEEP), E, W), BF16),
            pltpu.VMEM((NI * BS + 1, G, 8, W), BF16),
            pltpu.VMEM((NO, BS, G, 8, W), BF16),
            pltpu.VMEM((9 * C + 8, 128), F32),
            pltpu.VMEM((E // 2, 128), U32),
            pltpu.VMEM((C // 2, E), U32),
            pltpu.VMEM((C, 128), F32),
            pltpu.SMEM((1,), jnp.int32),
            pltpu.SemaphoreType.DMA((NI,)),
            pltpu.SemaphoreType.DMA((NO,)),
            pltpu.SemaphoreType.DMA((5,)),
        ],
        compiler_params=pltpu.CompilerParams(
            vmem_limit_bytes=128 * 1024 * 1024,
            disable_bounds_checks=True,
            flags={"XLA_TPU_RESCHEDULE_DMA_DONES": True},
        ),
        name="convnext",
    )(xt, dw, w1, w2.T, grn_gamma, grn_beta)
    return jnp.transpose(out.reshape(B, H, C, W), (0, 1, 3, 2))
```
